```python
import os as _os
_os.environ.setdefault("JAX_PLATFORMS", "cpu")
import jax
import jax.numpy as jnp

def _softmax(x, axis=-1):
    return jax.nn.softmax(x, axis=axis)
def _gelu(x):
    return jax.nn.gelu(x, approximate=True)
def _silu(x):
    return jax.nn.silu(x)
def _sigmoid(x):
    return jax.nn.sigmoid(x)
def _layernorm(x, axis=-1, eps=1e-5):
    m = jnp.mean(x, axis=axis, keepdims=True)
    v = jnp.var(x, axis=axis, keepdims=True)
    return (x - m) / jnp.sqrt(v + eps)
def _scatter_add(tgt, idx, src, axis=0):
    return tgt.at[idx].add(src)
def _segment_sum(src, seg, n):
    return jax.ops.segment_sum(src, seg, n)
class _Rng:
    def __init__(self, key):
        self._k = key
    def _next(self):
        self._k, sub = jax.random.split(self._k)
        return sub
    def normal(self, shape):
        return jax.random.normal(self._next(), shape, dtype=jnp.bfloat16)
    def randint(self, lo, hi, shape):
        return jax.random.randint(self._next(), shape, lo, hi, dtype=jnp.int32)
    def uniform(self, shape, lo=0.0, hi=1.0):
        return jax.random.uniform(self._next(), shape, jnp.bfloat16, lo, hi)
    def permutation(self, n):
        return jax.random.permutation(self._next(), n)


kernel_name = 'gated_mix__linear_kernel_hedgehog__glu_gated_bilinear__prompt'

def setup_inputs():
    _rng = _Rng(jax.random.key(int.from_bytes(__import__("os").urandom(4), "little")))
    _w = (lambda a: (lambda t: t.astype(jnp.bfloat16) if jnp.issubdtype(t.dtype, jnp.floating) else t)(jnp.asarray(a)))
    def _A_setup():
        B, S, D, H = 1, 2048, 512, 32
        Dh = D // H
        return {
            "x": _w((lambda *s: _rng.normal(s) * 0.05)(B, S, D)),
            "wqkv": _w((lambda *s: _rng.normal(s) * 0.8)(D, 3 * D)),
            "w_phi": _w((lambda *s: _rng.normal(s) * 0.8)(H, Dh, Dh) * (Dh ** -0.5)),
            "wo": _w((lambda *s: _rng.normal(s) * 0.05)(D, D)),
        }
    _A_in = _A_setup()

    def _B_setup():
        B, S, D, F = 1, 2048, 512, 1792
        return {
            "x": _w((lambda *s: _rng.normal(s) * 0.05)(B, S, D)),
            "w_gate": _w((lambda *s: _rng.normal(s) * 1.6)(D, F) * (D ** -0.5)),
            "w_up": _w((lambda *s: _rng.normal(s) * 1.6)(D, F) * (D ** -0.5)),
            "w_down": _w((lambda *s: _rng.normal(s) * 1.6)(F, D) * (F ** -0.5)),
        }
    _B_in = _B_setup()

    return {
        "A_x": _A_in["x"],
        "A_wqkv": _A_in["wqkv"],
        "A_w_phi": _A_in["w_phi"],
        "A_wo": _A_in["wo"],
        "B_x": _B_in["x"],
        "B_w_gate": _B_in["w_gate"],
        "B_w_up": _B_in["w_up"],
        "B_w_down": _B_in["w_down"],
        "gate_w": _w((lambda *s: _rng.normal(s) * 0.05)(512) * 16.0),
    }

def reference(A_x, A_wqkv, A_w_phi, A_wo, B_x, B_w_gate, B_w_up, B_w_down, gate_w):
    def _A_ref(x, wqkv, w_phi, wo):
        B, S, D = x.shape
        H = 32; Dh = D // H
        qkv = (lambda x, *d: x.transpose(*d))((x @ wqkv).reshape(B, S, 3, H, Dh), 2, 0, 3, 1, 4)
        q, k, v = qkv[0], qkv[1], qkv[2]
        pq = jnp.einsum("bhsd,hdf->bhsf", q, w_phi)
        pk = jnp.einsum("bhsd,hdf->bhsf", k, w_phi)
        phi_q = jnp.concatenate([_softmax(pq, axis=-1), _softmax(-pq, axis=-1)], axis=-1)
        phi_k = jnp.concatenate([_softmax(pk, axis=-1), _softmax(-pk, axis=-1)], axis=-1)
        kv = jnp.einsum("bhsf,bhsd->bhfd", phi_k, v)
        z  = jnp.einsum("bhsf->bhf", phi_k)
        num = jnp.einsum("bhqf,bhfd->bhqd", phi_q, kv)
        den = jnp.einsum("bhqf,bhf->bhq", phi_q, z)[..., None] + 1e-6
        o = num / den
        return (lambda x, *d: x.transpose(*d))(o, 0, 2, 1, 3).reshape(B, S, D) @ wo

    def _B_ref(x, w_gate, w_up, w_down):
        g = jnp.einsum("bsd,df->bsf", x, w_gate)
        u = jnp.einsum("bsd,df->bsf", x, w_up)
        h = g * u
        return jnp.einsum("bsf,fd->bsd", h, w_down)

    x = A_x
    g = _sigmoid((x * gate_w).sum(-1, keepdims=True))
    a = _A_ref(x, A_wqkv, A_w_phi, A_wo)
    b = _B_ref(x, B_w_gate, B_w_up, B_w_down)
    return g * a + (1 - g) * b
```

```python
import functools
import jax
import jax.numpy as jnp
from jax import lax
import jax.experimental.pallas as pl
import jax.experimental.pallas.tpu as pltpu

S, D, H, DH, F = 2048, 512, 32, 16, 1792
T1 = 512
T2 = 512
XC = 256
NXC = S // XC
NG = 8
BF = jnp.bfloat16
F32 = jnp.float32
NT_DIMS = (((1,), (1,)), ((), ()))


def _iota(shape, dim):
    return lax.broadcasted_iota(jnp.int32, shape, dim)


def _fold(x):
    return pltpu.roll(x, 4, axis=0)


def _dual_softmax_parts(pT):
    T = pT.shape[-1]
    p3 = pT.reshape(8, 8, T)
    mx = jnp.max(p3, axis=0)
    mx = jnp.maximum(mx, _fold(mx))
    mn = jnp.min(p3, axis=0)
    mn = jnp.minimum(mn, _fold(mn))
    e_pos = jnp.exp(p3 - mx[None])
    e_neg = jnp.exp(mn[None] - p3)
    s_pos = jnp.sum(e_pos, axis=0)
    s_pos = s_pos + _fold(s_pos)
    s_neg = jnp.sum(e_neg, axis=0)
    s_neg = s_neg + _fold(s_neg)
    return e_pos, e_neg, s_pos, s_neg


def _kernel(x_hbm, wqkv_hbm, wphi_hbm, wo_hbm, wg_hbm, wu_hbm, wd_hbm, gw_hbm, o_hbm,
            x_v, wqkv_v, wphi_v, wo_v, wg_v, wu_v, wd_v, gw_v, out_v,
            wqT_v, wkvT_v, kv_acc, z_acc, kvT_v, zb_v,
            sem_w, sem_x, sem_o):
    def cp(src, dst, sem):
        return pltpu.make_async_copy(src, dst, sem)

    c_phi = cp(wphi_hbm, wphi_v, sem_w.at[0])
    c_k = cp(wqkv_hbm.at[:, D:2 * D], wqkv_v.at[:, D:2 * D], sem_w.at[1])
    c_v = cp(wqkv_hbm.at[:, 2 * D:3 * D], wqkv_v.at[:, 2 * D:3 * D], sem_w.at[2])
    c_q = cp(wqkv_hbm.at[:, 0:D], wqkv_v.at[:, 0:D], sem_w.at[3])
    c_g = cp(wg_hbm, wg_v, sem_w.at[4])
    c_u = cp(wu_hbm, wu_v, sem_w.at[5])
    c_d = cp(wd_hbm, wd_v, sem_w.at[6])
    c_o = cp(wo_hbm, wo_v, sem_w.at[7])
    c_gw = cp(gw_hbm, gw_v, sem_w.at[8])

    def c_x(j):
        return cp(x_hbm.at[pl.ds(j * XC, XC)], x_v.at[pl.ds(j * XC, XC)], sem_x.at[j])

    c_phi.start()
    c_k.start()
    c_v.start()
    for j in range(NXC):
        c_x(j).start()
    c_q.start()
    c_gw.start()
    c_g.start()
    c_u.start()
    c_d.start()
    c_o.start()

    c_phi.wait()
    r = _iota((D, H), 0)
    c = _iota((D, H), 1)
    rsel = jnp.where(c == (r >> 6) * 4 + (r & 3), 1.0, 0.0).astype(BF)
    a = lax.dot_general(rsel, wphi_v[...], NT_DIMS, preferred_element_type=F32)
    r = _iota((D, 256), 0)
    c = _iota((D, 256), 1)
    a = jnp.where(((r >> 2) & 15) == (c & 15), a, 0.0).astype(BF)
    r = _iota((256, 128), 0)
    c = _iota((256, 128), 1)
    csel = jnp.where((r >> 4) == (c & 15), 1.0, 0.0).astype(BF)
    pt = jnp.dot(a, csel, preferred_element_type=F32)
    r = _iota((D, 128), 0)
    c = _iota((D, 128), 1)
    pt = jnp.where((c >> 4) == ((r >> 6) & 1) * 4 + (r & 3), pt, 0.0).astype(BF)

    kv_acc[...] = jnp.zeros(kv_acc.shape, F32)
    z_acc[...] = jnp.zeros(z_acc.shape, F32)

    c_k.wait()
    for g in range(4):
        wk = wqkv_v[:, D + g * 128:D + (g + 1) * 128]
        wkvT_v[g * 128:(g + 1) * 128, :] = lax.dot_general(
            pt[g * 128:(g + 1) * 128], wk, NT_DIMS, preferred_element_type=F32).astype(BF)
    c_v.wait()
    wkvT_v[D:2 * D, :] = wqkv_v[:, 2 * D:3 * D].astype(F32).T.astype(BF)

    def kside(i, carry):
        for jj in range(T1 // XC):
            c_x(i * (T1 // XC) + jj).wait()
        x = x_v[pl.ds(pl.multiple_of(i * T1, T1), T1), :]
        pv = lax.dot_general(wkvT_v[...], x, NT_DIMS, preferred_element_type=F32)
        for g in range(NG):
            e_pos, e_neg, s_pos, s_neg = _dual_softmax_parts(pv[g * 64:(g + 1) * 64])
            ph_pos = (e_pos * (1.0 / s_pos)[None]).reshape(64, T1)
            ph_neg = (e_neg * (1.0 / s_neg)[None]).reshape(64, T1)
            ph = jnp.concatenate([ph_pos, ph_neg], axis=0)
            zs = ph[:, 0:128]
            for j in range(1, T1 // 128):
                zs = zs + ph[:, j * 128:(j + 1) * 128]
            z_acc[g] += zs
            vT = pv[D + g * 64:D + (g + 1) * 64].astype(BF)
            kv_acc[g] += lax.dot_general(vT, ph.astype(BF), NT_DIMS, preferred_element_type=F32)
        return carry

    lax.fori_loop(0, S // T1, kside, 0)

    c_q.wait()
    for g in range(4):
        wq = wqkv_v[:, g * 128:(g + 1) * 128]
        wqT_v[g * 128:(g + 1) * 128, :] = lax.dot_general(
            pt[g * 128:(g + 1) * 128], wq, NT_DIMS, preferred_element_type=F32).astype(BF)
    r = _iota((64, 128), 0)
    c = _iota((64, 128), 1)
    kmask = (r >> 4) == (c & 3)
    for g in range(NG):
        kvT_v[g] = jnp.where(kmask, kv_acc[g], 0.0).astype(BF)
        zsum = jnp.sum(z_acc[g], axis=1, keepdims=True)
        zb_v[g] = jnp.broadcast_to(zsum, (128, 128))
    c_gw.wait()
    c_g.wait()
    c_u.wait()
    c_d.wait()
    c_o.wait()

    def c_out(i):
        return cp(out_v.at[pl.ds(i * T2, T2)], o_hbm.at[pl.ds(i * T2, T2)], sem_o.at[i])

    def qside(i, carry):
        row0 = pl.multiple_of(i * T2, T2)
        x = x_v[pl.ds(row0, T2), :]
        pqT = lax.dot_general(wqT_v[...], x, NT_DIMS, preferred_element_type=F32)
        gate = jnp.dot(x, wg_v[...], preferred_element_type=F32)
        oTs = []
        for g in range(NG):
            e_pos, e_neg, s_pos, s_neg = _dual_softmax_parts(pqT[g * 64:(g + 1) * 64])
            zb = zb_v[g]
            zb = jnp.concatenate([zb] * (T2 // 128), axis=1)
            z_pos = zb[0:64].reshape(8, 8, T2)
            z_neg = zb[64:128].reshape(8, 8, T2)
            r_pos = 1.0 / s_pos
            r_neg = 1.0 / s_neg
            den = jnp.sum(e_pos * z_pos, axis=0) * r_pos + jnp.sum(e_neg * z_neg, axis=0) * r_neg
            den = den + _fold(den) + 1e-6
            rd = 1.0 / den
            ph_pos = (e_pos * (r_pos * rd)[None]).reshape(64, T2)
            ph_neg = (e_neg * (r_neg * rd)[None]).reshape(64, T2)
            ph = jnp.concatenate([ph_pos, ph_neg], axis=0).astype(BF)
            oTs.append(jnp.dot(kvT_v[g], ph, preferred_element_type=F32))
        oT = jnp.concatenate(oTs, axis=0)
        o = oT.T.astype(BF)
        up = jnp.dot(x, wu_v[...], preferred_element_type=F32)
        h = (gate * up).astype(BF)
        a = jnp.dot(o, wo_v[...], preferred_element_type=F32)
        gw = gw_v[...].astype(F32)
        xf = x.astype(F32)
        lg = xf[:, 0:128] * gw[0:1]
        for j in range(1, 4):
            lg = lg + xf[:, j * 128:(j + 1) * 128] * gw[j:j + 1]
        logit = jnp.sum(lg, axis=1, keepdims=True)
        gt = 1.0 / (1.0 + jnp.exp(-logit))
        b = jnp.dot(h, wd_v[...], preferred_element_type=F32)
        out_v[pl.ds(row0, T2), :] = (b + gt * (a - b)).astype(BF)
        c_out(i).start()
        return carry

    lax.fori_loop(0, S // T2, qside, 0)
    for i in range(S // T2):
        c_out(i).wait()


@jax.jit
def pallas_gated_mix__linear_kernel_hedgehog__glu_gated_bilinear__prompt_kernel(
    A_x, A_wqkv, A_w_phi, A_wo, B_x, B_w_gate, B_w_up, B_w_down, gate_w,
):
    x = A_x.reshape(S, D)
    wphi = jnp.transpose(A_w_phi, (1, 2, 0)).reshape(DH * DH, H)
    gw = gate_w.reshape(4, 128)
    any_spec = pl.BlockSpec(memory_space=pl.ANY)
    out = pl.pallas_call(
        _kernel,
        in_specs=[any_spec] * 8,
        out_specs=any_spec,
        out_shape=jax.ShapeDtypeStruct((S, D), BF),
        scratch_shapes=[
            pltpu.VMEM((S, D), BF), pltpu.VMEM((D, 3 * D), BF), pltpu.VMEM((DH * DH, H), BF),
            pltpu.VMEM((D, D), BF), pltpu.VMEM((D, F), BF), pltpu.VMEM((D, F), BF),
            pltpu.VMEM((F, D), BF), pltpu.VMEM((4, 128), BF), pltpu.VMEM((S, D), BF),
            pltpu.VMEM((D, D), BF), pltpu.VMEM((2 * D, D), BF),
            pltpu.VMEM((NG, 64, 128), F32), pltpu.VMEM((NG, 128, 128), F32),
            pltpu.VMEM((NG, 64, 128), BF), pltpu.VMEM((NG, 128, 128), F32),
            pltpu.SemaphoreType.DMA((9,)), pltpu.SemaphoreType.DMA((NXC,)),
            pltpu.SemaphoreType.DMA((S // T2,)),
        ],
        compiler_params=pltpu.CompilerParams(vmem_limit_bytes=100 * 1024 * 1024),
    )(x, A_wqkv, wphi, A_wo, B_w_gate, B_w_up, B_w_down, gw)
    return out.reshape(1, S, D)
```

```python
import bisect
import jax
import jax.numpy as jnp
from jax import lax
import jax.experimental.pallas as pl
import jax.experimental.pallas.tpu as pltpu

S, D, H, DH, F = 2048, 512, 32, 16, 1792
NJ = S // 128
TG = S // 4
OUT_TILES = (256,) * 7 + (128, 128)
WID = 2
JLAG = 8
SLAG = 24
LLAG = 12
TLAG = 40
KMODE = "copy"
TB = 2
CB = 4
T0 = 0
DT = 20
CBN = 3
PLAG = 3
QS0 = 8
BF = jnp.bfloat16
F32 = jnp.float32
NT_DIMS = (((1,), (1,)), ((), ()))
XCH = ((0, 256), (256, 1024), (1024, 2048))
LOG2E = 1.4426950408889634


def _iota(shape, dim):
    return lax.broadcasted_iota(jnp.int32, shape, dim)


def _nt(a, b):
    return lax.dot_general(a, b, NT_DIMS, preferred_element_type=F32)


def _dot(a, b):
    return jnp.dot(a, b, preferred_element_type=F32)


def _dual_exp(p3, gate=None):
    mx = jnp.max(p3, axis=0)
    mn = jnp.min(p3, axis=0)
    if gate is not None:
        mx = gate(mx)
        mn = gate(mn)
    e_pos = jnp.exp2(p3 - mx[None])
    e_neg = jnp.exp2(mn[None] - p3)
    r_pos = 1.0 / jnp.sum(e_pos, axis=0)
    r_neg = 1.0 / jnp.sum(e_neg, axis=0)
    return e_pos.reshape(128, 128), e_neg.reshape(128, 128), r_pos, r_neg


def _kernel(x_hbm, wqkv_hbm, wphi_hbm, wo_hbm, wg_hbm, wu_hbm, wd_hbm, gw_hbm, o_hbm,
            x_v, wqkv_v, wphi_v, wo_v, wg_v, wu_v, wd_v, gw_v, out_v,
            pt_v, wkT_v, wvT_v, tmp_v, pk_v, ek_v, rk_v, vT_v, ot_v, o_v, bb_v, gt_v, zero_v, junk_v, es_v,
            sem_i, sem_o):
    def cp(src, dst, sem):
        return pltpu.make_async_copy(src, dst, sem)

    c_phi = cp(wphi_hbm, wphi_v, sem_i.at[0])
    c_k = cp(wqkv_hbm.at[:, D:2 * D], wqkv_v.at[:, D:2 * D], sem_i.at[1])
    c_v = cp(wqkv_hbm.at[:, 2 * D:3 * D], wqkv_v.at[:, 2 * D:3 * D], sem_i.at[2])
    c_q = cp(wqkv_hbm.at[:, 0:D], wqkv_v.at[:, 0:D], sem_i.at[3])
    c_g = cp(wg_hbm, wg_v, sem_i.at[4])
    c_u = cp(wu_hbm, wu_v, sem_i.at[5])
    c_d = cp(wd_hbm, wd_v, sem_i.at[6])
    c_o = cp(wo_hbm, wo_v, sem_i.at[7])
    c_gw = cp(gw_hbm, gw_v, sem_i.at[8])
    c_x = [cp(x_hbm.at[lo:hi], x_v.at[lo:hi], sem_i.at[9 + n]) for n, (lo, hi) in enumerate(XCH)]

    for c in (c_phi, c_k, c_x[0], c_x[1], c_x[2], c_v, c_gw, c_q, c_g, c_u, c_d, c_o):
        c.start()
    zero_v[...] = jnp.zeros(zero_v.shape, F32)

    c_phi.wait()
    r = _iota((D, H), 0)
    c = _iota((D, H), 1)
    rsel = jnp.where(c == (r >> 7) * 8 + (r & 7), 1.0, 0.0).astype(BF)
    a = _nt(rsel, wphi_v[...])
    r = _iota((D, 256), 0)
    c = _iota((D, 256), 1)
    a = jnp.where(((r >> 3) & 15) == (c & 15), a, 0.0).astype(BF)
    r = _iota((256, 128), 0)
    c = _iota((256, 128), 1)
    csel = jnp.where((r >> 4) == (c & 15), 1.0, 0.0).astype(BF)
    pt = _dot(a, csel)
    r = _iota((D, 128), 0)
    c = _iota((D, 128), 1)
    pt = jnp.where((c >> 4) == (r & 7), pt, 0.0).astype(BF)
    for g in range(4):
        pt_v[g] = pt[g * 128:(g + 1) * 128]

    c_k.wait()
    for g in range(4):
        wk = wqkv_v[:, D + g * 128:D + (g + 1) * 128]
        wkT_v[g * 128:(g + 1) * 128, :] = (_nt(pt[g * 128:(g + 1) * 128], wk) * LOG2E).astype(BF)

    def store_kexp(j, p3, gate=None):
        e_pos, e_neg, r_pos, r_neg = _dual_exp(p3, gate)
        ek_v[j, 0:128, :] = e_pos
        ek_v[j, 128:256, :] = e_neg
        rk_v[j, 0:8, :] = r_pos
        rk_v[j, 8:16, :] = r_neg
        return jnp.maximum(r_pos, r_neg)

    def kproj(lo, hi, toks=()):
        toks = list(toks)
        never = zero_v[...] != 0.0
        for t0 in range(lo, hi, 256):
            pk = _nt(wkT_v[...], x_v[t0:t0 + 256, :])
            for jj in range(2):
                j = t0 // 128 + jj
                store_kexp(j, pk[0:128, jj * 128:(jj + 1) * 128].reshape(16, 8, 128))
                for g in range(1, 4):
                    blk = pk[g * 128:(g + 1) * 128, jj * 128:(jj + 1) * 128]
                    if toks and t0 > lo:
                        blk = jnp.concatenate([jnp.where(never, toks.pop(0), blk[0:8]), blk[8:]], axis=0)
                    if KMODE == "exp":
                        pk_v[g - 1, j] = blk
                    else:
                        e_pos, e_neg, r_pos, r_neg = _dual_exp(blk.reshape(16, 8, 128))
                        es_v[g - 1, j, 0:128, :] = e_pos
                        es_v[g - 1, j, 128:256, :] = e_neg
                        es_v[g - 1, j, 256:264, :] = r_pos
                        es_v[g - 1, j, 264:272, :] = r_neg

    c_x[0].wait()
    kproj(*XCH[0])
    c_x[1].wait()
    kproj(*XCH[1])
    c_x[2].wait()
    c_v.wait()
    wv_toks = []
    for cc in range(4):
        tmp_v[cc] = wqkv_v[cc * 128:(cc + 1) * 128, 2 * D:3 * D].astype(F32).T
        for g in range(4):
            blk = jnp.concatenate(
                [tmp_v[cc, pl.ds(g * 128 + d, 8, stride=16), :] for d in range(16)], axis=0)
            wvT_v[g * 128:(g + 1) * 128, cc * 128:(cc + 1) * 128] = blk.astype(BF)
            tk = blk[0:8]
            for d in range(1, 16):
                tk = jnp.maximum(tk, blk[d * 8:(d + 1) * 8])
            wv_toks.append(tk)
    kproj(*XCH[2], toks=wv_toks)
    for t0 in range(0, S, 256):
        vt = _nt(wvT_v[...], x_v[t0:t0 + 256, :])
        for g in range(4):
            for jj in range(2):
                vT_v[g, t0 // 128 + jj] = vt[g * 128:(g + 1) * 128, jj * 128:(jj + 1) * 128]

    c_gw.wait()
    c_q.wait()
    c_g.wait()
    c_u.wait()
    c_d.wait()

    def body(g, carry):
        row0 = pl.multiple_of(g * TG, TG)
        col0 = pl.multiple_of(g * 128, 128)
        gn = jnp.minimum(g, 2)
        x = x_v[pl.ds(row0, TG), :]

        wqT = (_nt(pt_v[g], wqkv_v[:, pl.ds(col0, 128)]) * LOG2E).astype(BF)
        toks = []
        clock = [128]

        def track(y, cyc_per_tile):
            rows, cols = y.shape
            for n in range(cols // 128):
                for r0 in range(0, rows, 8):
                    toks.append((clock[0] + cyc_per_tile * r0 // rows, y, r0, n * 128))
                clock[0] += cyc_per_tile
            return y

        gate0 = track(_dot(x, wg_v[:, 0:256]), TG)
        pq = [track(_nt(wqT, x_v[t0:t0 + 512, :]), 128) for t0 in range(0, S, 512)]
        gate = jnp.concatenate([gate0, track(_dot(x, wg_v[:, 256:F]), TG)], axis=1)
        h = (gate * track(_dot(x, wu_v[...]), TG)).astype(BF)
        b = None
        for k0 in range(0, F, 512):
            k1 = min(k0 + 512, F)
            y = track(_dot(h[:, k0:k1], wd_v[k0:k1, :]), TG * (k1 - k0) // 512)
            b = y if b is None else b + y
        tok_times = [t[0] for t in toks]

        def mxu_tok(t):
            i = max(bisect.bisect_right(tok_times, t) - 1, 0)
            _, y, r0, c0 = toks[i]
            return y[r0:r0 + 8, c0:c0 + 128]

        gw = gw_v[...].astype(F32)
        xf = x.astype(F32)
        lg = xf[:, 0:128] * gw[0:1]
        for j in range(1, 4):
            lg = lg + xf[:, j * 128:(j + 1) * 128] * gw[j:j + 1]
        logit = jnp.sum(lg, axis=1, keepdims=True)
        gt = 1.0 / (1.0 + jnp.exp(-logit))
        gt_v[pl.ds(row0, TG), :] = jnp.broadcast_to(gt, (TG, 128))
        bb_v[pl.ds(row0, TG), :] = b * (1.0 - gt)

        never = zero_v[...] != 0.0
        st = {"tok": zero_v[...], "c": 0}
        junk = []
        copies = []

        def lanesum(acc):
            return jnp.broadcast_to(jnp.sum(acc, axis=1, keepdims=True), (8, 128))

        def gate_now():
            tk = st["tok"]
            return lambda v: jnp.where(never, tk, v)

        def chain(terms, post=None):
            n = len(terms)
            st["tok"] = mxu_tok(T0 + DT * st["c"])
            st["c"] += 1
            acc = None
            for s0 in range(0, n, WID):
                part = None
                for i in range(s0, min(s0 + WID, n)):
                    a_i, b_i = terms[i]
                    if i == 0:
                        a_i = jnp.where(never, st["tok"], a_i)
                    elif junk and junk[0][0] <= st["c"]:
                        a_i = jnp.where(never, junk.pop(0)[1], a_i)
                    t = a_i * b_i
                    part = t if part is None else part + t
                acc = part if acc is None else acc + part
            for _ in range(CBN if st["c"] % CB == 0 else 0):
                if not copies:
                    break
                cj, cr = copies.pop(0)
                val = jnp.where(never, st["tok"], es_v[gn, cj, cr:cr + 8, :])
                if cr < 256:
                    ek_v[cj, cr:cr + 8, :] = val
                else:
                    rk_v[cj, cr - 256:cr - 248, :] = val
            ls = None
            if post == "ls":
                ls = lanesum(acc)
                junk.append((st["c"] + JLAG, ls))
                junk.sort(key=lambda e: e[0])
            return acc, ls

        coef = {}
        eq = {}
        rq = {}

        def qexp(j):
            p3 = pq[j // 4][:, (j % 4) * 128:(j % 4 + 1) * 128].reshape(16, 8, 128)
            e_pos, e_neg, r_pos, r_neg = _dual_exp(p3, gate_now())
            eq[j] = [e_pos[f * 8:(f + 1) * 8] for f in range(16)] + [e_neg[f * 8:(f + 1) * 8] for f in range(16)]
            ts = []
            for sg in range(2):
                t = None
                for f in range(16):
                    u = coef[-1, sg * 16 + f] * eq[j][sg * 16 + f]
                    t = u if t is None else t + u
                ts.append(t)
            rd = 1.0 / (ts[0] * r_pos + ts[1] * r_neg + 1e-6)
            rq[j] = (r_pos * rd, r_neg * rd)
            junk.append((st["c"] + SLAG, jnp.maximum(rq[j][0], rq[j][1])))
            junk.sort(key=lambda e: e[0])

        def kexp_next(j):
            rn = store_kexp(j, pk_v[gn, j].reshape(16, 8, 128), gate_now())
            junk.append((st["c"] + SLAG, rn))
            junk.sort(key=lambda e: e[0])

        ngrp = 0
        for d in range(-1, DH):
            for sg in range(2):
                if QS0 <= ngrp < QS0 + NJ:
                    qexp(ngrp - QS0)
                ngrp += 1
                res = [rk_v[j, sg * 8:(sg + 1) * 8, :] for j in range(NJ)]
                if d >= 0:
                    res = [vT_v[g, j, d * 8:(d + 1) * 8, :] * res[j] for j in range(NJ)]
                for f in range(16):
                    r0 = sg * 128 + f * 8
                    coef[d, sg * 16 + f] = chain([(ek_v[j, r0:r0 + 8, :], res[j]) for j in range(NJ)], post="ls")[1]

        if KMODE == "copy":
            copies.extend((cj, cr) for cj in range(NJ) for cr in range(0, 272, 8))
        for j in range(NJ):
            c_pos, c_neg = rq[j]
            part = []
            for d in range(DH):
                part.append(chain([(coef[d, f], eq[j][f]) for f in range(16)])[0] * c_pos)
                if PLAG:
                    junk.append((st["c"] + PLAG, part[-1]))
                    junk.sort(key=lambda e: e[0])
            if KMODE == "exp":
                kexp_next(j)
            last = None
            for d in range(DH):
                acc = chain([(coef[d, 16 + f], eq[j][16 + f]) for f in range(16)])[0]
                last = part[d] + acc * c_neg
                ot_v[j, pl.ds(d, 8, stride=16), :] = last
                if LLAG:
                    junk.append((st["c"] + LLAG, last))
                    junk.sort(key=lambda e: e[0])
        for j0 in range(0, NJ, TB):
            ob = jnp.concatenate([ot_v[j] for j in range(j0, j0 + TB)], axis=1).T
            o_v[g, j0 * 128:(j0 + TB) * 128, :] = ob.astype(BF)
        assert not copies
        if junk:
            jk = junk[0][1]
            for _, t in junk[1:]:
                jk = jnp.maximum(jk, t)
            junk_v[g] = jk
        return carry

    lax.fori_loop(0, 4, body, 0)

    c_o.wait()
    outs = []
    t0 = 0
    for n, to in enumerate(OUT_TILES):
        o = jnp.concatenate([o_v[g, t0:t0 + to, :] for g in range(4)], axis=1)
        a = _dot(o, wo_v[...])
        gt = gt_v[t0:t0 + to, :]
        gt = jnp.concatenate([gt] * 4, axis=1)
        out_v[t0:t0 + to, :] = (gt * a + bb_v[t0:t0 + to, :]).astype(BF)
        co = cp(out_v.at[t0:t0 + to], o_hbm.at[t0:t0 + to], sem_o.at[n])
        co.start()
        outs.append(co)
        t0 += to
    for co in outs:
        co.wait()


@jax.jit
def pallas_gated_mix__linear_kernel_hedgehog__glu_gated_bilinear__prompt_kernel(
    A_x, A_wqkv, A_w_phi, A_wo, B_x, B_w_gate, B_w_up, B_w_down, gate_w,
):
    x = A_x.reshape(S, D)
    wphi = jnp.transpose(A_w_phi, (1, 2, 0)).reshape(DH * DH, H)
    gw = gate_w.reshape(4, 128)
    any_spec = pl.BlockSpec(memory_space=pl.ANY)
    out = pl.pallas_call(
        _kernel,
        in_specs=[any_spec] * 8,
        out_specs=any_spec,
        out_shape=jax.ShapeDtypeStruct((S, D), BF),
        scratch_shapes=[
            pltpu.VMEM((S, D), BF), pltpu.VMEM((D, 3 * D), BF), pltpu.VMEM((DH * DH, H), BF),
            pltpu.VMEM((D, D), BF), pltpu.VMEM((D, F), BF), pltpu.VMEM((D, F), BF),
            pltpu.VMEM((F, D), BF), pltpu.VMEM((4, 128), BF), pltpu.VMEM((S, D), BF),
            pltpu.VMEM((4, 128, 128), BF),
            pltpu.VMEM((D, D), BF),
            pltpu.VMEM((D, D), BF),
            pltpu.VMEM((4, D, 128), F32),
            pltpu.VMEM((3, NJ, 128, 128), F32),
            pltpu.VMEM((NJ, 264, 128), F32),
            pltpu.VMEM((NJ, 24, 128), F32),
            pltpu.VMEM((4, NJ, 128, 128), F32),
            pltpu.VMEM((NJ, 128, 128), F32),
            pltpu.VMEM((4, S, 128), BF),
            pltpu.VMEM((S, D), F32),
            pltpu.VMEM((S, 128), F32),
            pltpu.VMEM((8, 128), F32),
            pltpu.VMEM((4, 8, 128), F32),
            pltpu.VMEM((3, NJ, 272, 128), F32),
            pltpu.SemaphoreType.DMA((9 + len(XCH),)),
            pltpu.SemaphoreType.DMA((len(OUT_TILES),)),
        ],
        compiler_params=pltpu.CompilerParams(vmem_limit_bytes=100 * 1024 * 1024),
    )(x, A_wqkv, wphi, A_wo, B_w_gate, B_w_up, B_w_down, gw)
    return out.reshape(1, S, D)
```

```python
import bisect

import jax
import jax.numpy as jnp
from jax import lax
import jax.experimental.pallas as pl
import jax.experimental.pallas.tpu as pltpu

S, D, H, DH, F = 2048, 512, 32, 16, 1792
NJ = S // 128
TG = S // 4
OUT_TILES = (256,) * 7 + (128, 64, 64)
XCH = ((0, 384), (384, 1152), (1152, 2048))
WID = 2
T0 = 0
DT = 20
JLAG = 8
SLAG = 32
PLAG = 3
LLAG = 3
QS0 = 8
CB = 1
CBN = 2
DEFER = 2
ER = 408
BF = jnp.bfloat16
F32 = jnp.float32
NT_DIMS = (((1,), (1,)), ((), ()))
LOG2E = 1.4426950408889634


def _iota(shape, dim):
    return lax.broadcasted_iota(jnp.int32, shape, dim)


def _nt(a, b):
    return lax.dot_general(a, b, NT_DIMS, preferred_element_type=F32)


def _dot(a, b):
    return jnp.dot(a, b, preferred_element_type=F32)


def _dual_exp(p, gate=None):
    p3 = p.reshape(16, 8, 128)
    mx = jnp.max(p3, axis=0)
    mn = jnp.min(p3, axis=0)
    if gate is not None:
        mx = gate(mx)
        mn = gate(mn)
    e_pos = jnp.exp2(p3 - mx[None])
    e_neg = jnp.exp2(mn[None] - p3)
    r_pos = 1.0 / jnp.sum(e_pos, axis=0)
    r_neg = 1.0 / jnp.sum(e_neg, axis=0)
    return e_pos.reshape(128, 128), e_neg.reshape(128, 128), r_pos, r_neg


def _kernel(x_hbm, wqkv_hbm, wphi_hbm, wo_hbm, wg_hbm, wu_hbm, wd_hbm, gw_hbm, o_hbm,
            x_v, wqkv_v, wphi_v, wo_v, wg_v, wu_v, wd_v, gw_v, out_v,
            pt_v, wkT_v, wvT_v, tmp_v, es_v, ot_v, o_v, bb_v, gt_v, zero_v, junk_v,
            sem):
    def cp(src, dst, s):
        return pltpu.make_async_copy(src, dst, sem.at[s])

    c_phi = cp(wphi_hbm, wphi_v, 0)
    c_k = cp(wqkv_hbm.at[:, D:2 * D], wqkv_v.at[:, D:2 * D], 1)
    c_x = [cp(x_hbm.at[lo:hi], x_v.at[lo:hi], 2 + n) for n, (lo, hi) in enumerate(XCH)]
    c_v = cp(wqkv_hbm.at[:, 2 * D:3 * D], wqkv_v.at[:, 2 * D:3 * D], 4)
    c_rest = [cp(gw_hbm, gw_v, 5), cp(wqkv_hbm.at[:, 0:D], wqkv_v.at[:, 0:D], 5),
              cp(wg_hbm, wg_v, 5), cp(wu_hbm, wu_v, 5), cp(wd_hbm, wd_v, 5)]
    c_o = cp(wo_hbm, wo_v, 6)

    for c in [c_phi, c_k] + c_x + [c_v] + c_rest + [c_o]:
        c.start()
    zero_v[...] = jnp.zeros(zero_v.shape, F32)

    c_phi.wait()
    r = _iota((D, H), 0)
    c = _iota((D, H), 1)
    rsel = jnp.where(c == (r >> 7) * 8 + (r & 7), 1.0, 0.0).astype(BF)
    a = _nt(rsel, wphi_v[...])
    r = _iota((D, 256), 0)
    c = _iota((D, 256), 1)
    a = jnp.where(((r >> 3) & 15) == (c & 15), a, 0.0).astype(BF)
    r = _iota((256, 128), 0)
    c = _iota((256, 128), 1)
    csel = jnp.where((r >> 4) == (c & 15), 1.0, 0.0).astype(BF)
    pt = _dot(a, csel)
    r = _iota((D, 128), 0)
    c = _iota((D, 128), 1)
    pt = jnp.where((c >> 4) == (r & 7), pt, 0.0).astype(BF)
    for g in range(4):
        pt_v[g] = pt[g * 128:(g + 1) * 128]

    c_k.wait()
    for g in range(4):
        wk = wqkv_v[:, D + g * 128:D + (g + 1) * 128]
        wkT_v[g * 128:(g + 1) * 128, :] = (_nt(pt[g * 128:(g + 1) * 128], wk) * LOG2E).astype(BF)

    def kexp(g, j, blk):
        e_pos, e_neg, r_pos, r_neg = _dual_exp(blk)
        es_v[g, j, 0:128, :] = e_pos
        es_v[g, j, 128:256, :] = e_neg
        es_v[g, j, 256:264, :] = r_pos
        es_v[g, j, 264:272, :] = r_neg

    def kproj(lo, hi, toks=(), defer=0):
        toks = list(toks)
        never = zero_v[...] != 0.0
        late = []
        t0 = lo
        while t0 < hi:
            w = 256 if hi - t0 >= 256 else 128
            pk = _nt(wkT_v[...], x_v[t0:t0 + w, :])
            for jj in range(w // 128):
                j = t0 // 128 + jj
                for g in range(4):
                    blk = pk[g * 128:(g + 1) * 128, jj * 128:(jj + 1) * 128]
                    if toks and t0 > lo:
                        blk = jnp.concatenate([jnp.where(never, toks.pop(0), blk[0:8]), blk[8:]], axis=0)
                    if (j + 1) * 128 == hi and g >= 4 - defer:
                        late.append((g, j, blk))
                    else:
                        kexp(g, j, blk)
            t0 += w
        return late

    c_x[0].wait()
    late = kproj(*XCH[0], defer=DEFER)
    c_x[1].wait()
    for e in late:
        kexp(*e)
    late = kproj(*XCH[1], defer=DEFER)
    c_x[2].wait()
    c_v.wait()
    for e in late:
        kexp(*e)
    wv_toks = []
    for cc in range(4):
        tmp_v[cc, 0:D, :] = wqkv_v[cc * 128:(cc + 1) * 128, 2 * D:3 * D].astype(F32).T
        for g in range(4):
            blk = jnp.concatenate(
                [tmp_v[cc, pl.ds(g * 128 + d, 8, stride=16), :] for d in range(16)], axis=0)
            wvT_v[g * 128:(g + 1) * 128, cc * 128:(cc + 1) * 128] = blk.astype(BF)
            tk = blk[0:8]
            for d in range(1, 16):
                tk = jnp.maximum(tk, blk[d * 8:(d + 1) * 8])
            wv_toks.append(tk)
    kproj(*XCH[2], toks=wv_toks)
    for t0 in range(0, S, 256):
        vt = _nt(wvT_v[...], x_v[t0:t0 + 256, :])
        for g in range(4):
            for jj in range(2):
                blk = vt[g * 128:(g + 1) * 128, jj * 128:(jj + 1) * 128]
                es_v[g, t0 // 128 + jj, 272:400, :] = blk

    for c in c_rest:
        c.wait()

    def body(g, carry):
        row0 = pl.multiple_of(g * TG, TG)
        col0 = pl.multiple_of(g * 128, 128)
        x = x_v[pl.ds(row0, TG), :]
        toks = []
        clock = [0]

        def track(y, cyc_per_tile):
            rows, cols = y.shape
            for n in range(cols // 128):
                for r0 in range(0, rows, 8):
                    toks.append((clock[0] + cyc_per_tile * r0 // rows, y, r0, n * 128))
                clock[0] += cyc_per_tile
            return y

        gate0 = track(_dot(x, wg_v[:, 0:128]), TG)
        wqT = (track(_nt(pt_v[g], wqkv_v[:, pl.ds(col0, 128)]), 32) * LOG2E).astype(BF)
        gate1 = track(_dot(x, wg_v[:, 128:256]), TG)
        pq = [track(_nt(wqT, x_v[t0:t0 + 512, :]), 128) for t0 in range(0, S, 512)]
        gate = jnp.concatenate([gate0, gate1, track(_dot(x, wg_v[:, 256:F]), TG)], axis=1)
        h = (gate * track(_dot(x, wu_v[...]), TG)).astype(BF)
        b = None
        for k0 in range(0, F, 512):
            k1 = min(k0 + 512, F)
            y = track(_dot(h[:, k0:k1], wd_v[k0:k1, :]), TG * (k1 - k0) // 512)
            b = y if b is None else b + y
        tok_times = [t[0] for t in toks]

        gw = gw_v[...].astype(F32)
        xf = x.astype(F32)
        lg = xf[:, 0:128] * gw[0:1]
        for j in range(1, 4):
            lg = lg + xf[:, j * 128:(j + 1) * 128] * gw[j:j + 1]
        logit = jnp.sum(lg, axis=1, keepdims=True)
        gt = 1.0 / (1.0 + jnp.exp(-logit))
        gt_v[pl.ds(row0, TG), :] = jnp.broadcast_to(gt, (TG, 128))
        bb_v[pl.ds(row0, TG), :] = b * (1.0 - gt)

        never = zero_v[...] != 0.0
        st = {"tok": None, "c": 0}
        junk = []
        rot = []

        def after(tok, v):
            return jnp.where(never, tok, v)

        def due(lag, v):
            junk.append((st["c"] + lag, v))
            junk.sort(key=lambda e: e[0])

        def tick():
            i = max(bisect.bisect_right(tok_times, T0 + DT * st["c"]) - 1, 0)
            _, y, r0, c0 = toks[i]
            st["tok"] = y[r0:r0 + 8, c0:c0 + 128]

        def chain(a3, b3):
            tick()
            st["c"] += 1
            head = [after(st["tok"], a3[0])]
            while junk and junk[0][0] <= st["c"]:
                head.append(after(junk.pop(0)[1], a3[len(head)]))
            a3 = jnp.concatenate([jnp.stack(head), a3[len(head):]], axis=0)
            p = a3 * b3
            if WID > 1:
                p = jnp.sum(p.reshape(16 // WID, WID, 8, 128), axis=1)
            acc = jnp.sum(p, axis=0)
            if rot and st["c"] % CB == 0:
                cj, cr = rot.pop(0)
                for k in range(CBN):
                    r0 = cr + 8 * k
                    es_v[0:3, cj, r0:r0 + 8, :] = after(st["tok"], es_v[1:4, cj, r0:r0 + 8, :])
            return acc

        coef = {}
        eq = {}
        cq = {}

        def qexp(j):
            tick()
            tk = st["tok"]
            e_pos, e_neg, r_pos, r_neg = _dual_exp(
                pq[j // 4][:, (j % 4) * 128:(j % 4 + 1) * 128], lambda v: after(tk, v))
            eq[j] = (e_pos.reshape(16, 8, 128), e_neg.reshape(16, 8, 128))
            t_pos = jnp.sum(coef[-1, 0] * eq[j][0], axis=0)
            t_neg = jnp.sum(coef[-1, 1] * eq[j][1], axis=0)
            rd = 1.0 / (t_pos * r_pos + t_neg * r_neg + 1e-6)
            cq[j] = (r_pos * rd, r_neg * rd)
            due(SLAG, jnp.maximum(cq[j][0], cq[j][1]))

        ngrp = 0
        for d in range(-1, DH):
            for sg in range(2):
                if QS0 <= ngrp < QS0 + NJ:
                    qexp(ngrp - QS0)
                ngrp += 1
                res = es_v[0, :, 256 + sg * 8:264 + sg * 8, :]
                if d >= 0:
                    res = es_v[0, :, 272 + d * 8:280 + d * 8, :] * res
                cfs = []
                for f in range(16):
                    r0 = sg * 128 + f * 8
                    acc = chain(es_v[0, :, r0:r0 + 8, :], res)
                    cfs.append(jnp.broadcast_to(jnp.sum(acc, axis=1, keepdims=True), (8, 128)))
                    due(JLAG, cfs[-1])
                coef[d, sg] = jnp.stack(cfs)

        rot.extend((cj, cr) for cj in range(NJ) for cr in range(0, 400, 8 * CBN))
        for j in range(NJ):
            c_pos, c_neg = cq[j]
            part = []
            for d in range(DH):
                part.append(chain(coef[d, 0], eq[j][0]) * c_pos)
                due(PLAG, part[-1])
            for d in range(DH):
                last = part[d] + chain(coef[d, 1], eq[j][1]) * c_neg
                ot_v[j, pl.ds(d, 8, stride=16), :] = last
                due(LLAG, last)
            if j % 2 == 1:
                ob = jnp.concatenate([ot_v[j - 1, 0:128, :], ot_v[j, 0:128, :]], axis=1).T
                o_v[g, (j - 1) * 128:(j + 1) * 128, :] = ob.astype(BF)
        assert not rot
        jk = junk[0][1]
        for _, t in junk[1:]:
            jk = jnp.maximum(jk, t)
        junk_v[g] = jk
        return carry

    lax.fori_loop(0, 4, body, 0)

    c_o.wait()
    outs = []
    t0 = 0
    for to in OUT_TILES:
        o = jnp.concatenate([o_v[g, t0:t0 + to, :] for g in range(4)], axis=1)
        a = _dot(o, wo_v[...])
        gt = gt_v[t0:t0 + to, :]
        gt = jnp.concatenate([gt] * 4, axis=1)
        out_v[t0:t0 + to, :] = (gt * a + bb_v[t0:t0 + to, :]).astype(BF)
        co = cp(out_v.at[t0:t0 + to], o_hbm.at[t0:t0 + to], 7)
        co.start()
        outs.append(co)
        t0 += to
    for co in outs:
        co.wait()


@jax.jit
def pallas_gated_mix__linear_kernel_hedgehog__glu_gated_bilinear__prompt_kernel(
    A_x, A_wqkv, A_w_phi, A_wo, B_x, B_w_gate, B_w_up, B_w_down, gate_w,
):
    x = A_x.reshape(S, D)
    wphi = jnp.transpose(A_w_phi, (1, 2, 0)).reshape(DH * DH, H)
    gw = gate_w.reshape(4, 128)
    any_spec = pl.BlockSpec(memory_space=pl.ANY)
    out = pl.pallas_call(
        _kernel,
        in_specs=[any_spec] * 8,
        out_specs=any_spec,
        out_shape=jax.ShapeDtypeStruct((S, D), BF),
        scratch_shapes=[
            pltpu.VMEM((S, D), BF), pltpu.VMEM((D, 3 * D), BF), pltpu.VMEM((DH * DH, H), BF),
            pltpu.VMEM((D, D), BF), pltpu.VMEM((D, F), BF), pltpu.VMEM((D, F), BF),
            pltpu.VMEM((F, D), BF), pltpu.VMEM((4, 128), BF), pltpu.VMEM((S, D), BF),
            pltpu.VMEM((4, 128, 128), BF),
            pltpu.VMEM((D, D), BF),
            pltpu.VMEM((D, D), BF),
            pltpu.VMEM((4, D + 16, 128), F32),
            pltpu.VMEM((4, NJ, ER, 128), F32),
            pltpu.VMEM((NJ, 144, 128), F32),
            pltpu.VMEM((4, S, 128), BF),
            pltpu.VMEM((S, D), F32),
            pltpu.VMEM((S, 128), F32),
            pltpu.VMEM((8, 128), F32),
            pltpu.VMEM((4, 8, 128), F32),
            pltpu.SemaphoreType.DMA((8,)),
        ],
        compiler_params=pltpu.CompilerParams(vmem_limit_bytes=100 * 1024 * 1024),
    )(x, A_wqkv, wphi, A_wo, B_w_gate, B_w_up, B_w_down, gw)
    return out.reshape(1, S, D)
```

```python
import bisect

import jax
import jax.numpy as jnp
from jax import lax
import jax.experimental.pallas as pl
import jax.experimental.pallas.tpu as pltpu

S, D, H, DH, F = 2048, 512, 32, 16, 1792
NJ = S // 128
TG = S // 4
OUT_TILES = (256,) * 7 + (128, 64, 64)
XCH = ((0, 384), (384, 1152), (1152, 2048))
WID = 2
T0 = 0
DT = 20
JLAG = 8
SLAG = 32
PLAG = 3
LLAG = 3
QS0 = 8
CB = 1
CBN = 2
DEFER = 2
ER = 392
BF = jnp.bfloat16
F32 = jnp.float32
NT_DIMS = (((1,), (1,)), ((), ()))
LOG2E = 1.4426950408889634


def _iota(shape, dim):
    return lax.broadcasted_iota(jnp.int32, shape, dim)


def _nt(a, b):
    return lax.dot_general(a, b, NT_DIMS, preferred_element_type=F32)


def _dot(a, b):
    return jnp.dot(a, b, preferred_element_type=F32)


def _dual_exp(p, gate=None):
    if p.shape[0] == 120:
        p = jnp.concatenate([jnp.zeros((8, 128), F32), p], axis=0)
    p3 = p.reshape(16, 8, 128)
    mx = jnp.max(p3, axis=0)
    mn = jnp.min(p3, axis=0)
    if gate is not None:
        mx = gate(mx)
        mn = gate(mn)
    e_pos = jnp.exp2(p3 - mx[None])
    e_neg = jnp.exp2(mn[None] - p3)
    r_pos = 1.0 / jnp.sum(e_pos, axis=0)
    r_neg = 1.0 / jnp.sum(e_neg, axis=0)
    return e_pos.reshape(128, 128), e_neg.reshape(128, 128), r_pos, r_neg


def _kernel(x_hbm, wqkv_hbm, wphi_hbm, wo_hbm, wg_hbm, wu_hbm, wd_hbm, gw_hbm, o_hbm,
            x_v, wqkv_v, wphi_v, wo_v, wg_v, wu_v, wd_v, gw_v, out_v,
            pt_v, wkT_v, wvT_v, wv15_v, tmp_v, es_v, ot_v, o_v, bb_v, gt_v, zero_v, junk_v,
            sem):
    def cp(src, dst, s):
        return pltpu.make_async_copy(src, dst, sem.at[s])

    c_phi = cp(wphi_hbm, wphi_v, 0)
    c_k = cp(wqkv_hbm.at[:, D:2 * D], wqkv_v.at[:, D:2 * D], 1)
    c_x = [cp(x_hbm.at[lo:hi], x_v.at[lo:hi], s) for s, (lo, hi) in zip((2, 3, 0), XCH)]
    c_v = cp(wqkv_hbm.at[:, 2 * D:3 * D], wqkv_v.at[:, 2 * D:3 * D], 0)
    c_rest = [cp(gw_hbm, gw_v, 1), cp(wqkv_hbm.at[:, 0:D], wqkv_v.at[:, 0:D], 1),
              cp(wg_hbm, wg_v, 1), cp(wu_hbm, wu_v, 1), cp(wd_hbm, wd_v, 1)]
    c_o = cp(wo_hbm, wo_v, 2)

    for c in (c_phi, c_k, c_x[0], c_x[1]):
        c.start()
    zero_v[...] = jnp.zeros(zero_v.shape, F32)

    c_phi.wait()
    c_x[2].start()
    c_v.start()
    r = _iota((D, H), 0)
    c = _iota((D, H), 1)
    rsel = jnp.where(c == (r >> 7) * 8 + (r & 7), 1.0, 0.0).astype(BF)
    a = _nt(rsel, wphi_v[...])
    r = _iota((D, 256), 0)
    c = _iota((D, 256), 1)
    a = jnp.where(((r >> 3) & 15) == (c & 15), a, 0.0).astype(BF)
    r = _iota((256, 128), 0)
    c = _iota((256, 128), 1)
    csel = jnp.where((r >> 4) == (c & 15), 1.0, 0.0).astype(BF)
    pt = _dot(a, csel)
    r = _iota((D, 128), 0)
    c = _iota((D, 128), 1)
    pt = jnp.where((c >> 4) == (r & 7), pt, 0.0).astype(BF)
    for g in range(4):
        pt_v[g] = pt[g * 128:(g + 1) * 128]

    c_k.wait()
    for c in c_rest:
        c.start()
    rows = []
    for g in range(4):
        wk = wqkv_v[:, D + g * 128:D + (g + 1) * 128]
        w3 = _nt(pt[g * 128:(g + 1) * 128], wk).reshape(16, 8, D)
        rows.append(((w3[1:] - w3[0:1]) * LOG2E).reshape(120, D))
    wkT_v[...] = jnp.concatenate(rows, axis=0).astype(BF)

    def kexp(g, j, blk):
        e_pos, e_neg, r_pos, r_neg = _dual_exp(blk)
        es_v[g, j, 0:128, :] = e_pos
        es_v[g, j, 128:256, :] = e_neg
        es_v[g, j, 256:264, :] = r_pos
        es_v[g, j, 264:272, :] = r_neg

    def kproj(lo, hi, toks=(), defer=0):
        toks = list(toks)
        never = zero_v[...] != 0.0
        late = []
        t0 = lo
        while t0 < hi:
            w = 256 if hi - t0 >= 256 else 128
            pk = _nt(wkT_v[...], x_v[t0:t0 + w, :])
            for jj in range(w // 128):
                j = t0 // 128 + jj
                for g in range(4):
                    blk = pk[g * 120:(g + 1) * 120, jj * 128:(jj + 1) * 128]
                    if toks and t0 > lo:
                        blk = jnp.concatenate([jnp.where(never, toks.pop(0), blk[0:8]), blk[8:]], axis=0)
                    if (j + 1) * 128 == hi and g >= 4 - defer:
                        late.append((g, j, blk))
                    else:
                        kexp(g, j, blk)
            t0 += w
        return late

    c_x[0].wait()
    c_o.start()
    late = kproj(*XCH[0], defer=DEFER)
    c_x[1].wait()
    for e in late:
        kexp(*e)
    late = kproj(*XCH[1], defer=DEFER)
    c_x[2].wait()
    c_v.wait()
    for e in late:
        kexp(*e)
    wv_toks = []
    for cc in range(4):
        wvs = []
        tmp_v[cc, 0:D, :] = wqkv_v[cc * 128:(cc + 1) * 128, 2 * D:3 * D].astype(F32).T
        for g in range(4):
            blk = jnp.concatenate(
                [tmp_v[cc, pl.ds(g * 128 + d, 8, stride=16), :] for d in range(16)], axis=0)
            wvs.append(blk[0:120])
            wv15_v[g, :, cc * 128:(cc + 1) * 128] = blk[120:128]
            tk = blk[0:8]
            for d in range(1, 16):
                tk = jnp.maximum(tk, blk[d * 8:(d + 1) * 8])
            wv_toks.append(tk)
        wvT_v[:, cc * 128:(cc + 1) * 128] = jnp.concatenate(wvs, axis=0).astype(BF)
    kproj(*XCH[2], toks=wv_toks)
    for t0 in range(0, S, 256):
        vt = _nt(wvT_v[...], x_v[t0:t0 + 256, :])
        for g in range(4):
            for jj in range(2):
                blk = vt[g * 120:(g + 1) * 120, jj * 128:(jj + 1) * 128]
                es_v[g, t0 // 128 + jj, 272:392, :] = blk

    for c in c_rest:
        c.wait()

    def body(g, carry):
        row0 = pl.multiple_of(g * TG, TG)
        col0 = pl.multiple_of(g * 128, 128)
        x = x_v[pl.ds(row0, TG), :]
        toks = []
        clock = [0]

        def track(y, cyc_per_tile):
            rows, cols = y.shape
            for n in range(cols // 128):
                for r0 in range(0, rows, 8):
                    toks.append((clock[0] + cyc_per_tile * r0 // rows, y, r0, n * 128))
                clock[0] += cyc_per_tile
            return y

        gate0 = track(_dot(x, wg_v[:, 0:128]), TG)
        w3 = track(_nt(pt_v[g], wqkv_v[:, pl.ds(col0, 128)]), 32).reshape(16, 8, D)
        wqT = jnp.concatenate(
            [((w3[1:] - w3[0:1]) * LOG2E).reshape(120, D), wv15_v[g]], axis=0).astype(BF)
        gate1 = track(_dot(x, wg_v[:, 128:256]), TG)
        pq = [track(_nt(wqT, x_v[t0:t0 + 512, :]), 128) for t0 in range(0, S, 512)]
        gate = jnp.concatenate([gate0, gate1, track(_dot(x, wg_v[:, 256:F]), TG)], axis=1)
        h = (gate * track(_dot(x, wu_v[...]), TG)).astype(BF)
        b = None
        for k0 in range(0, F, 512):
            k1 = min(k0 + 512, F)
            y = track(_dot(h[:, k0:k1], wd_v[k0:k1, :]), TG * (k1 - k0) // 512)
            b = y if b is None else b + y
        tok_times = [t[0] for t in toks]

        gw = gw_v[...].astype(F32)
        xf = x.astype(F32)
        lg = xf[:, 0:128] * gw[0:1]
        for j in range(1, 4):
            lg = lg + xf[:, j * 128:(j + 1) * 128] * gw[j:j + 1]
        logit = jnp.sum(lg, axis=1, keepdims=True)
        gt = 1.0 / (1.0 + jnp.exp(-logit))
        gt_v[pl.ds(row0, TG), :] = jnp.broadcast_to(gt, (TG, 128))
        bb_v[pl.ds(row0, TG), :] = b * (1.0 - gt)

        never = zero_v[...] != 0.0
        st = {"tok": None, "c": 0}
        junk = []
        rot = []

        def after(tok, v):
            return jnp.where(never, tok, v)

        def due(lag, v):
            junk.append((st["c"] + lag, v))
            junk.sort(key=lambda e: e[0])

        def tick():
            i = max(bisect.bisect_right(tok_times, T0 + DT * st["c"]) - 1, 0)
            _, y, r0, c0 = toks[i]
            st["tok"] = y[r0:r0 + 8, c0:c0 + 128]

        def chain(a3, b3, nrot=0):
            tick()
            st["c"] += 1
            head = [after(st["tok"], a3[0])]
            while junk and junk[0][0] <= st["c"]:
                head.append(after(junk.pop(0)[1], a3[len(head)]))
            a3 = jnp.concatenate([jnp.stack(head), a3[len(head):]], axis=0)
            p = a3 * b3
            if WID > 1:
                p = jnp.sum(p.reshape(16 // WID, WID, 8, 128), axis=1)
            acc = jnp.sum(p, axis=0)
            for _ in range(nrot):
                if rot:
                    cj, r0 = rot.pop(0)
                    es_v[0:3, cj, r0:r0 + 8, :] = after(acc, es_v[1:4, cj, r0:r0 + 8, :])
            return acc

        coef = {}
        eq = {}
        cq = {}

        def qexp(j):
            tick()
            tk = st["tok"]
            e_pos, e_neg, r_pos, r_neg = _dual_exp(
                pq[j // 4][0:120, (j % 4) * 128:(j % 4 + 1) * 128], lambda v: after(tk, v))
            eq[j] = (e_pos.reshape(16, 8, 128), e_neg.reshape(16, 8, 128))
            t_pos = jnp.sum(coef[-1, 0] * eq[j][0], axis=0)
            t_neg = jnp.sum(coef[-1, 1] * eq[j][1], axis=0)
            rd = 1.0 / (t_pos * r_pos + t_neg * r_neg + 1e-6)
            cq[j] = (r_pos * rd, r_neg * rd)
            due(SLAG, jnp.maximum(cq[j][0], cq[j][1]))

        ngrp = 0
        for d in range(-1, DH):
            for sg in range(2):
                if QS0 <= ngrp < QS0 + NJ:
                    qexp(ngrp - QS0)
                ngrp += 1
                res = es_v[0, :, 256 + sg * 8:264 + sg * 8, :]
                if d == DH - 1:
                    res = jnp.stack([pq[j // 4][120:128, (j % 4) * 128:(j % 4 + 1) * 128]
                                     for j in range(NJ)]) * res
                elif d >= 0:
                    res = es_v[0, :, 272 + d * 8:280 + d * 8, :] * res
                cfs = []
                for f in range(16):
                    r0 = sg * 128 + f * 8
                    acc = chain(es_v[0, :, r0:r0 + 8, :], res)
                    cfs.append(jnp.broadcast_to(jnp.sum(acc, axis=1, keepdims=True), (8, 128)))
                    due(JLAG, cfs[-1])
                coef[d, sg] = jnp.stack(cfs)

        rot.extend((cj, cr) for cj in range(NJ) for cr in range(0, 392, 8))
        for j in range(NJ):
            c_pos, c_neg = cq[j]
            part = []
            for d in range(DH):
                part.append(chain(coef[d, 0], eq[j][0], nrot=2) * c_pos)
                if PLAG:
                    due(PLAG, part[-1])
            for d in range(DH):
                last = part[d] + chain(coef[d, 1], eq[j][1], nrot=2 if d == 0 else 1) * c_neg
                ot_v[j, pl.ds(d, 8, stride=16), :] = last
                if LLAG:
                    due(LLAG, last)
            if j % 2 == 1:
                ob = jnp.concatenate([ot_v[j - 1, 0:128, :], ot_v[j, 0:128, :]], axis=1).T
                o_v[g, (j - 1) * 128:(j + 1) * 128, :] = ob.astype(BF)
        assert not rot
        if junk:
            jk = junk[0][1]
            for _, t in junk[1:]:
                jk = jnp.maximum(jk, t)
            junk_v[g] = jk
        return carry

    lax.fori_loop(0, 4, body, 0)

    c_o.wait()
    outs = []
    t0 = 0
    for to in OUT_TILES:
        o = jnp.concatenate([o_v[g, t0:t0 + to, :] for g in range(4)], axis=1)
        a = _dot(o, wo_v[...])
        gt = gt_v[t0:t0 + to, :]
        gt = jnp.concatenate([gt] * 4, axis=1)
        out_v[t0:t0 + to, :] = (gt * a + bb_v[t0:t0 + to, :]).astype(BF)
        co = cp(out_v.at[t0:t0 + to], o_hbm.at[t0:t0 + to], 3)
        co.start()
        outs.append(co)
        t0 += to
    for co in outs:
        co.wait()


@jax.jit
def pallas_gated_mix__linear_kernel_hedgehog__glu_gated_bilinear__prompt_kernel(
    A_x, A_wqkv, A_w_phi, A_wo, B_x, B_w_gate, B_w_up, B_w_down, gate_w,
):
    x = A_x.reshape(S, D)
    wphi = jnp.transpose(A_w_phi, (1, 2, 0)).reshape(DH * DH, H)
    gw = gate_w.reshape(4, 128)
    any_spec = pl.BlockSpec(memory_space=pl.ANY)
    out = pl.pallas_call(
        _kernel,
        in_specs=[any_spec] * 8,
        out_specs=any_spec,
        out_shape=jax.ShapeDtypeStruct((S, D), BF),
        scratch_shapes=[
            pltpu.VMEM((S, D), BF), pltpu.VMEM((D, 3 * D), BF), pltpu.VMEM((DH * DH, H), BF),
            pltpu.VMEM((D, D), BF), pltpu.VMEM((D, F), BF), pltpu.VMEM((D, F), BF),
            pltpu.VMEM((F, D), BF), pltpu.VMEM((4, 128), BF), pltpu.VMEM((S, D), BF),
            pltpu.VMEM((4, 128, 128), BF),
            pltpu.VMEM((480, D), BF),
            pltpu.VMEM((480, D), BF),
            pltpu.VMEM((4, 8, D), F32),
            pltpu.VMEM((4, D + 16, 128), F32),
            pltpu.VMEM((4, NJ, ER, 128), F32),
            pltpu.VMEM((NJ, 144, 128), F32),
            pltpu.VMEM((4, S, 128), BF),
            pltpu.VMEM((S, D), F32),
            pltpu.VMEM((S, 128), F32),
            pltpu.VMEM((8, 128), F32),
            pltpu.VMEM((4, 8, 128), F32),
            pltpu.SemaphoreType.DMA((4,)),
        ],
        compiler_params=pltpu.CompilerParams(vmem_limit_bytes=100 * 1024 * 1024),
    )(x, A_wqkv, wphi, A_wo, B_w_gate, B_w_up, B_w_down, gw)
    return out.reshape(1, S, D)
```

```python
import bisect

import jax
import jax.numpy as jnp
from jax import lax
import jax.experimental.pallas as pl
import jax.experimental.pallas.tpu as pltpu

S, D, H, DH, F = 2048, 512, 32, 16, 1792
NJ = S // 128
TG = S // 4
OUT_TILES = (256,) * 7 + (128, 64, 64)
XCH = ((0, 384), (384, 1152), (1152, 2048))
DT = 20
JLAG = 8
SLAG = 32
PLAG = 3
QS0 = 8
DEFER = 2
ER = 392
BF = jnp.bfloat16
F32 = jnp.float32
NT_DIMS = (((1,), (1,)), ((), ()))
LOG2E = 1.4426950408889634


def _iota(shape, dim):
    return lax.broadcasted_iota(jnp.int32, shape, dim)


def _nt(a, b):
    return lax.dot_general(a, b, NT_DIMS, preferred_element_type=F32)


def _dot(a, b):
    return jnp.dot(a, b, preferred_element_type=F32)


def _rel_rows(w):
    w3 = w.reshape(16, 8, D)
    return ((w3[1:] - w3[0:1]) * LOG2E).reshape(120, D)


def _dual_exp(p, gate=None):
    p3 = jnp.concatenate([jnp.zeros((8, 128), F32), p], axis=0).reshape(16, 8, 128)
    mx = jnp.max(p3, axis=0)
    mn = jnp.min(p3, axis=0)
    if gate is not None:
        mx = gate(mx)
        mn = gate(mn)
    e_pos = jnp.exp2(p3 - mx[None])
    e_neg = jnp.exp2(mn[None] - p3)
    r_pos = 1.0 / jnp.sum(e_pos, axis=0)
    r_neg = 1.0 / jnp.sum(e_neg, axis=0)
    return e_pos, e_neg, r_pos, r_neg


def _kernel(x_hbm, wqkv_hbm, wphi_hbm, wo_hbm, wg_hbm, wu_hbm, wd_hbm, gw_hbm, o_hbm,
            x_v, wqkv_v, wphi_v, wo_v, wg_v, wu_v, wd_v, gw_v, out_v,
            pt_v, wkT_v, wvT_v, wv15_v, tmp_v, es_v, ot_v, o_v, bb_v, gt_v, zero_v, junk_v,
            sem):
    def cp(src, dst, s):
        return pltpu.make_async_copy(src, dst, sem.at[s])

    c_phi = cp(wphi_hbm, wphi_v, 0)
    c_k = cp(wqkv_hbm.at[:, D:2 * D], wqkv_v.at[:, D:2 * D], 1)
    c_x = [cp(x_hbm.at[lo:hi], x_v.at[lo:hi], s) for s, (lo, hi) in zip((2, 3, 0), XCH)]
    c_v = cp(wqkv_hbm.at[:, 2 * D:3 * D], wqkv_v.at[:, 2 * D:3 * D], 0)
    c_rest = [cp(gw_hbm, gw_v, 1), cp(wqkv_hbm.at[:, 0:D], wqkv_v.at[:, 0:D], 1),
              cp(wg_hbm, wg_v, 1), cp(wu_hbm, wu_v, 1), cp(wd_hbm, wd_v, 1)]
    c_o = cp(wo_hbm, wo_v, 2)

    for c in (c_phi, c_k, c_x[0], c_x[1]):
        c.start()
    zero_v[...] = jnp.zeros(zero_v.shape, F32)

    c_phi.wait()
    c_x[2].start()
    c_v.start()
    r = _iota((D, H), 0)
    c = _iota((D, H), 1)
    rsel = jnp.where(c == (r >> 7) * 8 + (r & 7), 1.0, 0.0).astype(BF)
    a = _nt(rsel, wphi_v[...])
    r = _iota((D, 256), 0)
    c = _iota((D, 256), 1)
    a = jnp.where(((r >> 3) & 15) == (c & 15), a, 0.0).astype(BF)
    r = _iota((256, 128), 0)
    c = _iota((256, 128), 1)
    csel = jnp.where((r >> 4) == (c & 15), 1.0, 0.0).astype(BF)
    pt = _dot(a, csel)
    r = _iota((D, 128), 0)
    c = _iota((D, 128), 1)
    pt = jnp.where((c >> 4) == (r & 7), pt, 0.0).astype(BF)
    for g in range(4):
        pt_v[g] = pt[g * 128:(g + 1) * 128]

    c_k.wait()
    for c in c_rest:
        c.start()
    rows = []
    for g in range(4):
        wk = wqkv_v[:, D + g * 128:D + (g + 1) * 128]
        rows.append(_rel_rows(_nt(pt[g * 128:(g + 1) * 128], wk)))
    wkT_v[...] = jnp.concatenate(rows, axis=0).astype(BF)

    def kexp(g, j, blk):
        e_pos, e_neg, r_pos, r_neg = _dual_exp(blk)
        es_v[g, j, 0:128, :] = e_pos.reshape(128, 128)
        es_v[g, j, 128:256, :] = e_neg.reshape(128, 128)
        es_v[g, j, 256:264, :] = r_pos
        es_v[g, j, 264:272, :] = r_neg

    def kproj(lo, hi, toks=(), defer=0):
        toks = list(toks)
        never = zero_v[...] != 0.0
        late = []
        t0 = lo
        while t0 < hi:
            w = 256 if hi - t0 >= 256 else 128
            pk = _nt(wkT_v[...], x_v[t0:t0 + w, :])
            for jj in range(w // 128):
                j = t0 // 128 + jj
                for g in range(4):
                    blk = pk[g * 120:(g + 1) * 120, jj * 128:(jj + 1) * 128]
                    if toks and t0 > lo:
                        blk = jnp.concatenate([jnp.where(never, toks.pop(0), blk[0:8]), blk[8:]], axis=0)
                    if (j + 1) * 128 == hi and g >= 4 - defer:
                        late.append((g, j, blk))
                    else:
                        kexp(g, j, blk)
            t0 += w
        return late

    c_x[0].wait()
    c_o.start()
    late = kproj(*XCH[0], defer=DEFER)
    c_x[1].wait()
    for e in late:
        kexp(*e)
    late = kproj(*XCH[1], defer=DEFER)
    c_x[2].wait()
    c_v.wait()
    for e in late:
        kexp(*e)
    wv_toks = []
    for cc in range(4):
        wvs = []
        tmp_v[cc, 0:D, :] = wqkv_v[cc * 128:(cc + 1) * 128, 2 * D:3 * D].astype(F32).T
        for g in range(4):
            blk = jnp.concatenate(
                [tmp_v[cc, pl.ds(g * 128 + d, 8, stride=16), :] for d in range(16)], axis=0)
            wvs.append(blk[0:120])
            wv15_v[g, :, cc * 128:(cc + 1) * 128] = blk[120:128]
            tk = blk[0:8]
            for d in range(1, 16):
                tk = jnp.maximum(tk, blk[d * 8:(d + 1) * 8])
            wv_toks.append(tk)
        wvT_v[:, cc * 128:(cc + 1) * 128] = jnp.concatenate(wvs, axis=0).astype(BF)
    kproj(*XCH[2], toks=wv_toks)
    for t0 in range(0, S, 256):
        vt = _nt(wvT_v[...], x_v[t0:t0 + 256, :])
        for g in range(4):
            for jj in range(2):
                es_v[g, t0 // 128 + jj, 272:392, :] = vt[g * 120:(g + 1) * 120, jj * 128:(jj + 1) * 128]

    for c in c_rest:
        c.wait()

    def body(g, carry):
        row0 = pl.multiple_of(g * TG, TG)
        col0 = pl.multiple_of(g * 128, 128)
        x = x_v[pl.ds(row0, TG), :]
        toks = []
        clock = [0]

        def track(y, cyc_per_tile):
            nr, nc = y.shape
            for n in range(nc // 128):
                for r0 in range(0, nr, 8):
                    toks.append((clock[0] + cyc_per_tile * r0 // nr, y, r0, n * 128))
                clock[0] += cyc_per_tile
            return y

        gate0 = track(_dot(x, wg_v[:, 0:128]), TG)
        wq = track(_nt(pt_v[g], wqkv_v[:, pl.ds(col0, 128)]), 32)
        wqT = jnp.concatenate([_rel_rows(wq), wv15_v[g]], axis=0).astype(BF)
        gate1 = track(_dot(x, wg_v[:, 128:256]), TG)
        pq = [track(_nt(wqT, x_v[t0:t0 + 512, :]), 128) for t0 in range(0, S, 512)]
        gate = jnp.concatenate([gate0, gate1, track(_dot(x, wg_v[:, 256:F]), TG)], axis=1)
        h = (gate * track(_dot(x, wu_v[...]), TG)).astype(BF)
        b = None
        for k0 in range(0, F, 512):
            k1 = min(k0 + 512, F)
            y = track(_dot(h[:, k0:k1], wd_v[k0:k1, :]), TG * (k1 - k0) // 512)
            b = y if b is None else b + y
        tok_times = [t[0] for t in toks]

        gw = gw_v[...].astype(F32)
        xf = x.astype(F32)
        lg = xf[:, 0:128] * gw[0:1]
        for j in range(1, 4):
            lg = lg + xf[:, j * 128:(j + 1) * 128] * gw[j:j + 1]
        logit = jnp.sum(lg, axis=1, keepdims=True)
        gt = 1.0 / (1.0 + jnp.exp(-logit))
        gt_v[pl.ds(row0, TG), :] = jnp.broadcast_to(gt, (TG, 128))
        bb_v[pl.ds(row0, TG), :] = b * (1.0 - gt)

        never = zero_v[...] != 0.0
        st = {"tok": None, "c": 0}
        junk = []
        rot = []

        def after(tok, v):
            return jnp.where(never, tok, v)

        def due(lag, v):
            junk.append((st["c"] + lag, v))
            junk.sort(key=lambda e: e[0])

        def tick():
            i = max(bisect.bisect_right(tok_times, DT * st["c"]) - 1, 0)
            _, y, r0, c0 = toks[i]
            st["tok"] = y[r0:r0 + 8, c0:c0 + 128]

        def chain(a3, b3, nrot=0):
            tick()
            st["c"] += 1
            head = [after(st["tok"], a3[0])]
            while junk and junk[0][0] <= st["c"]:
                head.append(after(junk.pop(0)[1], a3[len(head)]))
            a3 = jnp.concatenate([jnp.stack(head), a3[len(head):]], axis=0)
            p = jnp.sum((a3 * b3).reshape(8, 2, 8, 128), axis=1)
            acc = jnp.sum(p, axis=0)
            for _ in range(nrot):
                if rot:
                    cj, r0 = rot.pop(0)
                    es_v[0:3, cj, r0:r0 + 8, :] = after(acc, es_v[1:4, cj, r0:r0 + 8, :])
            return acc

        coef = {}
        eq = {}
        cq = {}

        def qexp(j):
            tick()
            tk = st["tok"]
            e_pos, e_neg, r_pos, r_neg = _dual_exp(
                pq[j // 4][0:120, (j % 4) * 128:(j % 4 + 1) * 128], lambda v: after(tk, v))
            eq[j] = (e_pos, e_neg)
            t_pos = jnp.sum(coef[-1, 0] * e_pos, axis=0)
            t_neg = jnp.sum(coef[-1, 1] * e_neg, axis=0)
            rd = 1.0 / (t_pos * r_pos + t_neg * r_neg + 1e-6)
            cq[j] = (r_pos * rd, r_neg * rd)
            due(SLAG, jnp.maximum(cq[j][0], cq[j][1]))

        ngrp = 0
        for d in range(-1, DH):
            for sg in range(2):
                if QS0 <= ngrp < QS0 + NJ:
                    qexp(ngrp - QS0)
                ngrp += 1
                res = es_v[0, :, 256 + sg * 8:264 + sg * 8, :]
                if d == DH - 1:
                    res = jnp.stack([pq[j // 4][120:128, (j % 4) * 128:(j % 4 + 1) * 128]
                                     for j in range(NJ)]) * res
                elif d >= 0:
                    res = es_v[0, :, 272 + d * 8:280 + d * 8, :] * res
                cfs = []
                for f in range(16):
                    r0 = sg * 128 + f * 8
                    acc = chain(es_v[0, :, r0:r0 + 8, :], res)
                    cfs.append(jnp.broadcast_to(jnp.sum(acc, axis=1, keepdims=True), (8, 128)))
                    due(JLAG, cfs[-1])
                coef[d, sg] = jnp.stack(cfs)

        rot.extend((cj, cr) for cj in range(NJ) for cr in range(0, ER, 8))
        for j in range(NJ):
            c_pos, c_neg = cq[j]
            part = []
            for d in range(DH):
                part.append(chain(coef[d, 0], eq[j][0], nrot=2) * c_pos)
                due(PLAG, part[-1])
            for d in range(DH):
                last = part[d] + chain(coef[d, 1], eq[j][1], nrot=2 if d == 0 else 1) * c_neg
                ot_v[j, pl.ds(d, 8, stride=16), :] = last
                due(PLAG, last)
            if j % 2 == 1:
                ob = jnp.concatenate([ot_v[j - 1, 0:128, :], ot_v[j, 0:128, :]], axis=1).T
                o_v[g, (j - 1) * 128:(j + 1) * 128, :] = ob.astype(BF)
        assert not rot
        jk = junk[0][1]
        for _, t in junk[1:]:
            jk = jnp.maximum(jk, t)
        junk_v[g] = jk
        return carry

    lax.fori_loop(0, 4, body, 0)

    c_o.wait()
    outs = []
    t0 = 0
    for to in OUT_TILES:
        o = jnp.concatenate([o_v[g, t0:t0 + to, :] for g in range(4)], axis=1)
        a = _dot(o, wo_v[...])
        gt = gt_v[t0:t0 + to, :]
        gt = jnp.concatenate([gt] * 4, axis=1)
        out_v[t0:t0 + to, :] = (gt * a + bb_v[t0:t0 + to, :]).astype(BF)
        co = cp(out_v.at[t0:t0 + to], o_hbm.at[t0:t0 + to], 3)
        co.start()
        outs.append(co)
        t0 += to
    for co in outs:
        co.wait()


@jax.jit
def pallas_gated_mix__linear_kernel_hedgehog__glu_gated_bilinear__prompt_kernel(
    A_x: jax.Array,
    A_wqkv: jax.Array,
    A_w_phi: jax.Array,
    A_wo: jax.Array,
    B_x: jax.Array,
    B_w_gate: jax.Array,
    B_w_up: jax.Array,
    B_w_down: jax.Array,
    gate_w: jax.Array,
):
    del B_x
    x = A_x.reshape(S, D)
    wphi = jnp.transpose(A_w_phi, (1, 2, 0)).reshape(DH * DH, H)
    gw = gate_w.reshape(4, 128)
    any_spec = pl.BlockSpec(memory_space=pl.ANY)
    out = pl.pallas_call(
        _kernel,
        in_specs=[any_spec] * 8,
        out_specs=any_spec,
        out_shape=jax.ShapeDtypeStruct((S, D), BF),
        scratch_shapes=[
            pltpu.VMEM((S, D), BF), pltpu.VMEM((D, 3 * D), BF), pltpu.VMEM((DH * DH, H), BF),
            pltpu.VMEM((D, D), BF), pltpu.VMEM((D, F), BF), pltpu.VMEM((D, F), BF),
            pltpu.VMEM((F, D), BF), pltpu.VMEM((4, 128), BF), pltpu.VMEM((S, D), BF),
            pltpu.VMEM((4, 128, 128), BF),
            pltpu.VMEM((480, D), BF),
            pltpu.VMEM((480, D), BF),
            pltpu.VMEM((4, 8, D), F32),
            pltpu.VMEM((4, D + 16, 128), F32),
            pltpu.VMEM((4, NJ, ER, 128), F32),
            pltpu.VMEM((NJ, 144, 128), F32),
            pltpu.VMEM((4, S, 128), BF),
            pltpu.VMEM((S, D), F32),
            pltpu.VMEM((S, 128), F32),
            pltpu.VMEM((8, 128), F32),
            pltpu.VMEM((4, 8, 128), F32),
            pltpu.SemaphoreType.DMA((4,)),
        ],
        compiler_params=pltpu.CompilerParams(vmem_limit_bytes=100 * 1024 * 1024),
    )(x, A_wqkv, wphi, A_wo, B_w_gate, B_w_up, B_w_down, gw)
    return out.reshape(1, S, D)
```

```python
import bisect

import jax
import jax.numpy as jnp
from jax import lax
import jax.experimental.pallas as pl
import jax.experimental.pallas.tpu as pltpu

S, D, H, DH, F = 2048, 512, 32, 16, 1792
NJ = S // 128
TG = S // 4
OUT_TILES = (256,) * 7 + (128, 64, 64)
XCH = ((0, 384), (384, 1152), (1152, 2048))
DT = 20
JLAG = 8
SLAG = 32
PLAG = 3
NG0 = 5
CW_TILES = 14
QS0 = 9
DEFER = 2
ER = 392
BF = jnp.bfloat16
F32 = jnp.float32
NT_DIMS = (((1,), (1,)), ((), ()))
LOG2E = 1.4426950408889634


def _iota(shape, dim):
    return lax.broadcasted_iota(jnp.int32, shape, dim)


def _nt(a, b):
    return lax.dot_general(a, b, NT_DIMS, preferred_element_type=F32)


def _dot(a, b):
    return jnp.dot(a, b, preferred_element_type=F32)


def _rel_rows(w):
    w3 = w.reshape(16, 8, D)
    return ((w3[1:] - w3[0:1]) * LOG2E).reshape(120, D)


def _dual_exp(p, gate=None):
    p3 = jnp.concatenate([jnp.zeros((8, 128), F32), p], axis=0).reshape(16, 8, 128)
    mx = jnp.max(p3, axis=0)
    mn = jnp.min(p3, axis=0)
    if gate is not None:
        mx = gate(mx)
        mn = gate(mn)
    e_pos = jnp.exp2(p3 - mx[None])
    e_neg = jnp.exp2(mn[None] - p3)
    r_pos = 1.0 / jnp.sum(e_pos, axis=0)
    r_neg = 1.0 / jnp.sum(e_neg, axis=0)
    return e_pos, e_neg, r_pos, r_neg


def _kernel(x_hbm, wqkv_hbm, wphi_hbm, wo_hbm, wg_hbm, wu_hbm, wd_hbm, gw_hbm, o_hbm,
            x_v, wqkv_v, wphi_v, wo_v, wg_v, wu_v, wd_v, gw_v, out_v,
            pt_v, wkT_v, wvT_v, wv15_v, tmp_v, es_v, ot_v, o_v, bb_v, gt_v, zero_v, junk_v, cw_v,
            sem):
    def cp(src, dst, s):
        return pltpu.make_async_copy(src, dst, sem.at[s])

    c_phi = cp(wphi_hbm, wphi_v, 0)
    c_k = cp(wqkv_hbm.at[:, D:2 * D], wqkv_v.at[:, D:2 * D], 1)
    c_x = [cp(x_hbm.at[lo:hi], x_v.at[lo:hi], s) for s, (lo, hi) in zip((2, 3, 0), XCH)]
    c_v = cp(wqkv_hbm.at[:, 2 * D:3 * D], wqkv_v.at[:, 2 * D:3 * D], 0)
    c_rest = [cp(gw_hbm, gw_v, 1), cp(wqkv_hbm.at[:, 0:D], wqkv_v.at[:, 0:D], 1),
              cp(wg_hbm, wg_v, 1), cp(wu_hbm, wu_v, 1), cp(wd_hbm, wd_v, 1)]
    c_o = cp(wo_hbm, wo_v, 2)

    for c in (c_phi, c_k, c_x[0], c_x[1]):
        c.start()
    zero_v[...] = jnp.zeros(zero_v.shape, F32)

    c_phi.wait()
    c_x[2].start()
    c_v.start()
    r = _iota((D, H), 0)
    c = _iota((D, H), 1)
    rsel = jnp.where(c == (r >> 7) * 8 + (r & 7), 1.0, 0.0).astype(BF)
    a = _nt(rsel, wphi_v[...])
    r = _iota((D, 256), 0)
    c = _iota((D, 256), 1)
    a = jnp.where(((r >> 3) & 15) == (c & 15), a, 0.0).astype(BF)
    r = _iota((256, 128), 0)
    c = _iota((256, 128), 1)
    csel = jnp.where((r >> 4) == (c & 15), 1.0, 0.0).astype(BF)
    pt = _dot(a, csel)
    r = _iota((D, 128), 0)
    c = _iota((D, 128), 1)
    pt = jnp.where((c >> 4) == (r & 7), pt, 0.0).astype(BF)
    for g in range(4):
        pt_v[g] = pt[g * 128:(g + 1) * 128]

    c_k.wait()
    for c in c_rest:
        c.start()
    rows = []
    for g in range(4):
        wk = wqkv_v[:, D + g * 128:D + (g + 1) * 128]
        rows.append(_rel_rows(_nt(pt[g * 128:(g + 1) * 128], wk)))
    wkT_v[...] = jnp.concatenate(rows, axis=0).astype(BF)

    def kexp(g, j, blk):
        e_pos, e_neg, r_pos, r_neg = _dual_exp(blk)
        es_v[g, j, 0:128, :] = e_pos.reshape(128, 128)
        es_v[g, j, 128:256, :] = e_neg.reshape(128, 128)
        es_v[g, j, 256:264, :] = r_pos
        es_v[g, j, 264:272, :] = r_neg

    def kproj(lo, hi, toks=(), defer=0):
        toks = list(toks)
        never = zero_v[...] != 0.0
        late = []
        t0 = lo
        while t0 < hi:
            w = 256 if hi - t0 >= 256 else 128
            pk = _nt(wkT_v[...], x_v[t0:t0 + w, :])
            for jj in range(w // 128):
                j = t0 // 128 + jj
                for g in range(4):
                    blk = pk[g * 120:(g + 1) * 120, jj * 128:(jj + 1) * 128]
                    if toks and t0 > lo:
                        blk = jnp.concatenate([jnp.where(never, toks.pop(0), blk[0:8]), blk[8:]], axis=0)
                    if (j + 1) * 128 == hi and g >= 4 - defer:
                        late.append((g, j, blk))
                    else:
                        kexp(g, j, blk)
            t0 += w
        return late

    c_x[0].wait()
    c_o.start()
    late = kproj(*XCH[0], defer=DEFER)
    c_x[1].wait()
    for e in late:
        kexp(*e)
    late = kproj(*XCH[1], defer=DEFER)
    c_x[2].wait()
    c_v.wait()
    for e in late:
        kexp(*e)
    wv_toks = []
    for cc in range(4):
        wvs = []
        tmp_v[cc, 0:D, :] = wqkv_v[cc * 128:(cc + 1) * 128, 2 * D:3 * D].astype(F32).T
        for g in range(4):
            blk = jnp.concatenate(
                [tmp_v[cc, pl.ds(g * 128 + d, 8, stride=16), :] for d in range(16)], axis=0)
            wvs.append(blk[0:120])
            wv15_v[g, :, cc * 128:(cc + 1) * 128] = blk[120:128]
            tk = blk[0:8]
            for d in range(1, 16):
                tk = jnp.maximum(tk, blk[d * 8:(d + 1) * 8])
            wv_toks.append(tk)
        wvT_v[:, cc * 128:(cc + 1) * 128] = jnp.concatenate(wvs, axis=0).astype(BF)
    kproj(*XCH[2], toks=wv_toks)
    vts = []
    for t0 in range(0, S, 256):
        vt = _nt(wvT_v[...], x_v[t0:t0 + 256, :])
        vts.append(vt)
        for g in range(4):
            for jj in range(2):
                es_v[g, t0 // 128 + jj, 272:392, :] = vt[g * 120:(g + 1) * 120, jj * 128:(jj + 1) * 128]
    never = zero_v[...] != 0.0
    lane = _iota((8, 128), 1) & 15
    for g in range(4):
        p3 = pt_v[g].astype(F32).reshape(16, 8, 128)
        for d in range(DH):
            n = g * DH + d
            tile = n * CW_TILES // 64
            frac = (n * CW_TILES % 64) * 56 // 64
            tk = vts[tile // 2][frac * 8:frac * 8 + 8, (tile % 2) * 128:(tile % 2 + 1) * 128]
            base = jnp.where(never, tk, p3[0])
            diff = jnp.where(lane == d, (p3[1:] - base[None]) * LOG2E, 0.0)
            cw_v[g, :, d * 8:(d + 1) * 8, :] = jnp.broadcast_to(
                jnp.sum(diff, axis=2, keepdims=True), (15, 8, 128))

    for c in c_rest:
        c.wait()

    def body(g, carry):
        row0 = pl.multiple_of(g * TG, TG)
        col0 = pl.multiple_of(g * 128, 128)
        x = x_v[pl.ds(row0, TG), :]
        toks = []
        clock = [0]

        def track(y, cyc_per_tile):
            nr, nc = y.shape
            for n in range(nc // 128):
                for r0 in range(0, nr, 8):
                    toks.append((clock[0] + cyc_per_tile * r0 // nr, y, r0, n * 128))
                clock[0] += cyc_per_tile
            return y

        gate0 = track(_dot(x, wg_v[:, 0:NG0 * 128]), TG)
        tok_times = [t[0] for t in toks]

        never = zero_v[...] != 0.0
        st = {"tok": None, "c": 0}
        junk = []
        rot = []

        def after(tok, v):
            return jnp.where(never, tok, v)

        def due(lag, v):
            junk.append((st["c"] + lag, v))
            junk.sort(key=lambda e: e[0])

        def tick():
            i = max(bisect.bisect_right(tok_times, DT * st["c"]) - 1, 0)
            _, y, r0, c0 = toks[i]
            st["tok"] = y[r0:r0 + 8, c0:c0 + 128]

        def chain(a3, b3, nrot=0):
            tick()
            st["c"] += 1
            head = [after(st["tok"], a3[0])]
            while junk and junk[0][0] <= st["c"]:
                head.append(after(junk.pop(0)[1], a3[len(head)]))
            a3 = jnp.concatenate([jnp.stack(head), a3[len(head):]], axis=0)
            p = jnp.sum((a3 * b3).reshape(8, 2, 8, 128), axis=1)
            acc = jnp.sum(p, axis=0)
            for _ in range(nrot):
                if rot:
                    ref, cj, r0 = rot.pop(0)
                    ref[0:3, cj, r0:r0 + 8, :] = after(acc, ref[1:4, cj, r0:r0 + 8, :])
            return acc

        wqt = wqkv_v[:, pl.ds(col0, 128)].astype(F32).T
        for cc in range(4):
            tmp_v[cc, 0:128, :] = wqt[:, cc * 128:(cc + 1) * 128]

        def kgroup(sg, res):
            cfs = []
            for f in range(16):
                r0 = sg * 128 + f * 8
                acc = chain(es_v[0, :, r0:r0 + 8, :], res)
                cfs.append(jnp.broadcast_to(jnp.sum(acc, axis=1, keepdims=True), (8, 128)))
                due(JLAG, cfs[-1])
            return jnp.stack(cfs)

        coef = {}
        for sg in range(2):
            coef[-1, sg] = kgroup(sg, es_v[0, :, 256 + sg * 8:264 + sg * 8, :])
        cols = []
        for cc in range(4):
            wd3 = jnp.stack([tmp_v[cc, pl.ds(d, 8, stride=16), :] for d in range(DH)])
            rows_c = []
            for f in range(15):
                rows_c.append(chain(cw_v[0, f].reshape(16, 8, 128), wd3))
                due(PLAG, rows_c[-1])
            cols.append(jnp.concatenate(rows_c, axis=0))
        wqT = jnp.concatenate([jnp.concatenate(cols, axis=1), wv15_v[g]], axis=0).astype(BF)

        pq = [track(_nt(wqT, x_v[t0:t0 + 512, :]), 128) for t0 in range(0, S, 512)]
        gate = jnp.concatenate([gate0, track(_dot(x, wg_v[:, NG0 * 128:F]), TG)], axis=1)
        h = (gate * track(_dot(x, wu_v[...]), TG)).astype(BF)
        b = None
        for k0 in range(0, F, 512):
            k1 = min(k0 + 512, F)
            y = track(_dot(h[:, k0:k1], wd_v[k0:k1, :]), TG * (k1 - k0) // 512)
            b = y if b is None else b + y
        tok_times[:] = [t[0] for t in toks]

        gw = gw_v[...].astype(F32)
        xf = x.astype(F32)
        lg = xf[:, 0:128] * gw[0:1]
        for j in range(1, 4):
            lg = lg + xf[:, j * 128:(j + 1) * 128] * gw[j:j + 1]
        logit = jnp.sum(lg, axis=1, keepdims=True)
        gt = 1.0 / (1.0 + jnp.exp(-logit))
        gt_v[pl.ds(row0, TG), :] = jnp.broadcast_to(gt, (TG, 128))
        bb_v[pl.ds(row0, TG), :] = b * (1.0 - gt)

        eq = {}
        cq = {}

        def qexp(j):
            tick()
            tk = st["tok"]
            e_pos, e_neg, r_pos, r_neg = _dual_exp(
                pq[j // 4][0:120, (j % 4) * 128:(j % 4 + 1) * 128], lambda v: after(tk, v))
            eq[j] = (e_pos, e_neg)
            t_pos = jnp.sum(coef[-1, 0] * e_pos, axis=0)
            t_neg = jnp.sum(coef[-1, 1] * e_neg, axis=0)
            rd = 1.0 / (t_pos * r_pos + t_neg * r_neg + 1e-6)
            cq[j] = (r_pos * rd, r_neg * rd)
            due(SLAG, jnp.maximum(cq[j][0], cq[j][1]))

        ngrp = 0
        for d in range(DH):
            for sg in range(2):
                if QS0 <= ngrp < QS0 + NJ:
                    qexp(ngrp - QS0)
                ngrp += 1
                res = es_v[0, :, 256 + sg * 8:264 + sg * 8, :]
                if d == DH - 1:
                    res = jnp.stack([pq[j // 4][120:128, (j % 4) * 128:(j % 4 + 1) * 128]
                                     for j in range(NJ)]) * res
                else:
                    res = es_v[0, :, 272 + d * 8:280 + d * 8, :] * res
                coef[d, sg] = kgroup(sg, res)

        rot.extend((es_v, cj, cr) for cj in range(NJ) for cr in range(0, ER, 8))
        rot.extend((cw_v, cj, cr) for cj in range(15) for cr in range(0, 128, 8))
        for j in range(NJ):
            c_pos, c_neg = cq[j]
            part = []
            for d in range(DH):
                part.append(chain(coef[d, 0], eq[j][0], nrot=2) * c_pos)
                due(PLAG, part[-1])
            for d in range(DH):
                last = part[d] + chain(coef[d, 1], eq[j][1], nrot=2) * c_neg
                ot_v[j, pl.ds(d, 8, stride=16), :] = last
                due(PLAG, last)
            if j % 2 == 1:
                ob = jnp.concatenate([ot_v[j - 1, 0:128, :], ot_v[j, 0:128, :]], axis=1).T
                o_v[g, (j - 1) * 128:(j + 1) * 128, :] = ob.astype(BF)
        assert not rot
        jk = junk[0][1]
        for _, t in junk[1:]:
            jk = jnp.maximum(jk, t)
        junk_v[g] = jk
        return carry

    lax.fori_loop(0, 4, body, 0)

    c_o.wait()
    outs = []
    t0 = 0
    for to in OUT_TILES:
        o = jnp.concatenate([o_v[g, t0:t0 + to, :] for g in range(4)], axis=1)
        a = _dot(o, wo_v[...])
        gt = gt_v[t0:t0 + to, :]
        gt = jnp.concatenate([gt] * 4, axis=1)
        out_v[t0:t0 + to, :] = (gt * a + bb_v[t0:t0 + to, :]).astype(BF)
        co = cp(out_v.at[t0:t0 + to], o_hbm.at[t0:t0 + to], 3)
        co.start()
        outs.append(co)
        t0 += to
    for co in outs:
        co.wait()


@jax.jit
def pallas_gated_mix__linear_kernel_hedgehog__glu_gated_bilinear__prompt_kernel(
    A_x: jax.Array,
    A_wqkv: jax.Array,
    A_w_phi: jax.Array,
    A_wo: jax.Array,
    B_x: jax.Array,
    B_w_gate: jax.Array,
    B_w_up: jax.Array,
    B_w_down: jax.Array,
    gate_w: jax.Array,
):
    del B_x
    x = A_x.reshape(S, D)
    wphi = jnp.transpose(A_w_phi, (1, 2, 0)).reshape(DH * DH, H)
    gw = gate_w.reshape(4, 128)
    any_spec = pl.BlockSpec(memory_space=pl.ANY)
    out = pl.pallas_call(
        _kernel,
        in_specs=[any_spec] * 8,
        out_specs=any_spec,
        out_shape=jax.ShapeDtypeStruct((S, D), BF),
        scratch_shapes=[
            pltpu.VMEM((S, D), BF), pltpu.VMEM((D, 3 * D), BF), pltpu.VMEM((DH * DH, H), BF),
            pltpu.VMEM((D, D), BF), pltpu.VMEM((D, F), BF), pltpu.VMEM((D, F), BF),
            pltpu.VMEM((F, D), BF), pltpu.VMEM((4, 128), BF), pltpu.VMEM((S, D), BF),
            pltpu.VMEM((4, 128, 128), BF),
            pltpu.VMEM((480, D), BF),
            pltpu.VMEM((480, D), BF),
            pltpu.VMEM((4, 8, D), F32),
            pltpu.VMEM((4, D + 16, 128), F32),
            pltpu.VMEM((4, NJ, ER, 128), F32),
            pltpu.VMEM((NJ, 144, 128), F32),
            pltpu.VMEM((4, S, 128), BF),
            pltpu.VMEM((S, D), F32),
            pltpu.VMEM((S, 128), F32),
            pltpu.VMEM((8, 128), F32),
            pltpu.VMEM((4, 8, 128), F32),
            pltpu.VMEM((4, 15, 128, 128), F32),
            pltpu.SemaphoreType.DMA((4,)),
        ],
        compiler_params=pltpu.CompilerParams(vmem_limit_bytes=100 * 1024 * 1024),
    )(x, A_wqkv, wphi, A_wo, B_w_gate, B_w_up, B_w_down, gw)
    return out.reshape(1, S, D)
```

```python
import bisect

import jax
import jax.numpy as jnp
from jax import lax
import jax.experimental.pallas as pl
import jax.experimental.pallas.tpu as pltpu

S, D, H, DH, F = 2048, 512, 32, 16, 1792
NJ = S // 128
TG = S // 4
OUT_TILES = (256,) * 7 + (128, 64, 64)
XCH = ((0, 384), (384, 1152), (1152, 2048))
DT = 20
JLAG = 8
SLAG = 32
PLAG = 3
NG0 = 5
CW_TILES = 14
QS0 = 9
DEFER = 2
ER = 392
BF = jnp.bfloat16
F32 = jnp.float32
NT_DIMS = (((1,), (1,)), ((), ()))
LOG2E = 1.4426950408889634


def _iota(shape, dim):
    return lax.broadcasted_iota(jnp.int32, shape, dim)


def _nt(a, b):
    return lax.dot_general(a, b, NT_DIMS, preferred_element_type=F32)


def _dot(a, b):
    return jnp.dot(a, b, preferred_element_type=F32)


def _stack(vs):
    return jnp.concatenate(vs, axis=0).reshape(len(vs), 8, 128)


def _rel_rows(w):
    w3 = w.reshape(16, 8, D)
    return ((w3[1:] - w3[0:1]) * LOG2E).reshape(120, D)


def _dual_exp(p, gate=None):
    p3 = jnp.concatenate([jnp.zeros((8, 128), F32), p], axis=0).reshape(16, 8, 128)
    mx = jnp.max(p3, axis=0)
    mn = jnp.min(p3, axis=0)
    if gate is not None:
        mx = gate(mx)
        mn = gate(mn)
    e_pos = jnp.exp2(p3 - mx[None])
    e_neg = jnp.exp2(mn[None] - p3)
    r_pos = 1.0 / jnp.sum(e_pos, axis=0)
    r_neg = 1.0 / jnp.sum(e_neg, axis=0)
    return e_pos, e_neg, r_pos, r_neg


def _kernel(x_hbm, wqkv_hbm, wphi_hbm, wo_hbm, wg_hbm, wu_hbm, wd_hbm, gw_hbm, o_hbm,
            x_v, wqkv_v, wphi_v, wo_v, wg_v, wu_v, wd_v, gw_v, out_v,
            pt_v, wkT_v, wvT_v, wv15_v, tmp_v, es_v, ot_v, o_v, bb_v, gt_v, zero_v, junk_v, cw_v,
            sem):
    def cp(src, dst, s):
        return pltpu.make_async_copy(src, dst, sem.at[s])

    c_phi = cp(wphi_hbm, wphi_v, 0)
    c_k = cp(wqkv_hbm.at[:, D:2 * D], wqkv_v.at[:, D:2 * D], 1)
    c_x = [cp(x_hbm.at[lo:hi], x_v.at[lo:hi], s) for s, (lo, hi) in zip((2, 3, 0), XCH)]
    c_v = cp(wqkv_hbm.at[:, 2 * D:3 * D], wqkv_v.at[:, 2 * D:3 * D], 0)
    c_rest = [cp(gw_hbm, gw_v, 1), cp(wqkv_hbm.at[:, 0:D], wqkv_v.at[:, 0:D], 1),
              cp(wg_hbm, wg_v, 1), cp(wu_hbm, wu_v, 1), cp(wd_hbm, wd_v, 1)]
    c_o = cp(wo_hbm, wo_v, 2)

    for c in (c_phi, c_k, c_x[0], c_x[1]):
        c.start()
    zero_v[...] = jnp.zeros(zero_v.shape, F32)
    ot_v[...] = jnp.zeros(ot_v.shape, F32)
    tmp_v[:, D:D + 16, :] = jnp.zeros((4, 16, 128), F32)

    c_phi.wait()
    c_x[2].start()
    c_v.start()
    r = _iota((D, H), 0)
    c = _iota((D, H), 1)
    rsel = jnp.where(c == (r >> 7) * 8 + (r & 7), 1.0, 0.0).astype(BF)
    a = _nt(rsel, wphi_v[...])
    r = _iota((D, 256), 0)
    c = _iota((D, 256), 1)
    a = jnp.where(((r >> 3) & 15) == (c & 15), a, 0.0).astype(BF)
    r = _iota((256, 128), 0)
    c = _iota((256, 128), 1)
    csel = jnp.where((r >> 4) == (c & 15), 1.0, 0.0).astype(BF)
    pt = _dot(a, csel)
    r = _iota((D, 128), 0)
    c = _iota((D, 128), 1)
    pt = jnp.where((c >> 4) == (r & 7), pt, 0.0).astype(BF)
    for g in range(4):
        pt_v[g] = pt[g * 128:(g + 1) * 128]

    c_k.wait()
    for c in c_rest:
        c.start()
    rows = []
    for g in range(4):
        wk = wqkv_v[:, D + g * 128:D + (g + 1) * 128]
        rows.append(_rel_rows(_nt(pt[g * 128:(g + 1) * 128], wk)))
    wkT_v[...] = jnp.concatenate(rows, axis=0).astype(BF)

    def kexp(g, j, blk):
        e_pos, e_neg, r_pos, r_neg = _dual_exp(blk)
        es_v[g, j, 0:128, :] = e_pos.reshape(128, 128)
        es_v[g, j, 128:256, :] = e_neg.reshape(128, 128)
        es_v[g, j, 256:264, :] = r_pos
        es_v[g, j, 264:272, :] = r_neg

    def kproj(lo, hi, toks=(), defer=0):
        toks = list(toks)
        never = zero_v[...] != 0.0
        late = []
        t0 = lo
        while t0 < hi:
            w = 256 if hi - t0 >= 256 else 128
            pk = _nt(wkT_v[...], x_v[t0:t0 + w, :])
            for jj in range(w // 128):
                j = t0 // 128 + jj
                for g in range(4):
                    blk = pk[g * 120:(g + 1) * 120, jj * 128:(jj + 1) * 128]
                    if toks and t0 > lo:
                        blk = jnp.concatenate([jnp.where(never, toks.pop(0), blk[0:8]), blk[8:]], axis=0)
                    if (j + 1) * 128 == hi and g >= 4 - defer:
                        late.append((g, j, blk))
                    else:
                        kexp(g, j, blk)
            t0 += w
        return late

    c_x[0].wait()
    c_o.start()
    late = kproj(*XCH[0], defer=DEFER)
    c_x[1].wait()
    for e in late:
        kexp(*e)
    late = kproj(*XCH[1], defer=DEFER)
    c_x[2].wait()
    c_v.wait()
    for e in late:
        kexp(*e)
    wv_toks = []
    for cc in range(4):
        wvs = []
        tmp_v[cc, 0:D, :] = wqkv_v[cc * 128:(cc + 1) * 128, 2 * D:3 * D].astype(F32).T
        for g in range(4):
            blk = jnp.concatenate(
                [tmp_v[cc, pl.ds(g * 128 + d, 8, stride=16), :] for d in range(16)], axis=0)
            wvs.append(blk[0:120])
            wv15_v[g, :, cc * 128:(cc + 1) * 128] = blk[120:128]
            tk = blk[0:8]
            for d in range(1, 16):
                tk = jnp.maximum(tk, blk[d * 8:(d + 1) * 8])
            wv_toks.append(tk)
        wvT_v[:, cc * 128:(cc + 1) * 128] = jnp.concatenate(wvs, axis=0).astype(BF)
    kproj(*XCH[2], toks=wv_toks)
    vts = []
    for t0 in range(0, S, 256):
        vt = _nt(wvT_v[...], x_v[t0:t0 + 256, :])
        vts.append(vt)
        for g in range(4):
            for jj in range(2):
                es_v[g, t0 // 128 + jj, 272:392, :] = vt[g * 120:(g + 1) * 120, jj * 128:(jj + 1) * 128]
    never = zero_v[...] != 0.0
    lane = _iota((8, 128), 1) & 15
    for g in range(4):
        p3 = pt_v[g].astype(F32).reshape(16, 8, 128)
        for d in range(DH):
            n = g * DH + d
            tile = n * CW_TILES // 64
            frac = (n * CW_TILES % 64) * 56 // 64
            tk = vts[tile // 2][frac * 8:frac * 8 + 8, (tile % 2) * 128:(tile % 2 + 1) * 128]
            base = jnp.where(never, tk, p3[0])
            diff = jnp.where(lane == d, (p3[1:] - base[None]) * LOG2E, 0.0)
            cw_v[g, :, d * 8:(d + 1) * 8, :] = jnp.broadcast_to(
                jnp.sum(diff, axis=2, keepdims=True), (15, 8, 128))

    for c in c_rest:
        c.wait()

    def body(g, carry):
        row0 = pl.multiple_of(g * TG, TG)
        col0 = pl.multiple_of(g * 128, 128)
        x = x_v[pl.ds(row0, TG), :]
        toks = []
        clock = [0]

        def track(y, cyc_per_tile):
            nr, nc = y.shape
            for n in range(nc // 128):
                for r0 in range(0, nr, 8):
                    toks.append((clock[0] + cyc_per_tile * r0 // nr, y, r0, n * 128))
                clock[0] += cyc_per_tile
            return y

        gate0 = track(_dot(x, wg_v[:, 0:NG0 * 128]), TG)
        tok_times = [t[0] for t in toks]

        never = zero_v[...] != 0.0
        st = {"tok": None, "c": 0}
        junk = []
        rot = []

        def after(tok, v):
            return jnp.where(never, tok, v)

        def due(lag, v):
            junk.append((st["c"] + lag, v))
            junk.sort(key=lambda e: e[0])

        def tick():
            i = max(bisect.bisect_right(tok_times, DT * st["c"]) - 1, 0)
            _, y, r0, c0 = toks[i]
            st["tok"] = y[r0:r0 + 8, c0:c0 + 128]

        def chain(a3, b3, nrot=0):
            tick()
            st["c"] += 1
            head = [after(st["tok"], a3[0])]
            while junk and junk[0][0] <= st["c"]:
                head.append(after(junk.pop(0)[1], a3[len(head)]))
            a3 = jnp.concatenate([v[None] for v in head] + [a3[len(head):]], axis=0)
            p = jnp.sum((a3 * b3).reshape(8, 2, 8, 128), axis=1)
            acc = jnp.sum(p, axis=0)
            for _ in range(nrot):
                if rot:
                    ref, cj, r0 = rot.pop(0)
                    ref[0:3, cj, r0:r0 + 8, :] = after(acc, ref[1:4, cj, r0:r0 + 8, :])
            return acc

        wqt = wqkv_v[:, pl.ds(col0, 128)].astype(F32).T
        for cc in range(4):
            tmp_v[cc, 0:128, :] = wqt[:, cc * 128:(cc + 1) * 128]

        def kgroup(sg, res):
            cfs = []
            for f in range(16):
                r0 = sg * 128 + f * 8
                acc = chain(es_v[0, :, r0:r0 + 8, :], res)
                cfs.append(jnp.broadcast_to(jnp.sum(acc, axis=1, keepdims=True), (8, 128)))
                due(JLAG, cfs[-1])
            return _stack(cfs)

        coef = {}
        for sg in range(2):
            coef[-1, sg] = kgroup(sg, es_v[0, :, 256 + sg * 8:264 + sg * 8, :])
        cols = []
        for cc in range(4):
            wd3 = _stack([tmp_v[cc, pl.ds(d, 8, stride=16), :] for d in range(DH)])
            rows_c = []
            for f in range(15):
                rows_c.append(chain(cw_v[0, f].reshape(16, 8, 128), wd3))
                due(PLAG, rows_c[-1])
            cols.append(jnp.concatenate(rows_c, axis=0))
        wqT = jnp.concatenate([jnp.concatenate(cols, axis=1), wv15_v[g]], axis=0).astype(BF)

        pq = [track(_nt(wqT, x_v[t0:t0 + 512, :]), 128) for t0 in range(0, S, 512)]
        gate = jnp.concatenate([gate0, track(_dot(x, wg_v[:, NG0 * 128:F]), TG)], axis=1)
        h = (gate * track(_dot(x, wu_v[...]), TG)).astype(BF)
        b = None
        for k0 in range(0, F, 512):
            k1 = min(k0 + 512, F)
            y = track(_dot(h[:, k0:k1], wd_v[k0:k1, :]), TG * (k1 - k0) // 512)
            b = y if b is None else b + y
        tok_times[:] = [t[0] for t in toks]

        gw = gw_v[...].astype(F32)
        xf = x.astype(F32)
        lg = xf[:, 0:128] * gw[0:1]
        for j in range(1, 4):
            lg = lg + xf[:, j * 128:(j + 1) * 128] * gw[j:j + 1]
        logit = jnp.sum(lg, axis=1, keepdims=True)
        gt = 1.0 / (1.0 + jnp.exp(-logit))
        gt_v[pl.ds(row0, TG), :] = jnp.broadcast_to(gt, (TG, 128))
        bb_v[pl.ds(row0, TG), :] = b * (1.0 - gt)

        eq = {}
        cq = {}

        def qexp(j):
            tick()
            tk = st["tok"]
            e_pos, e_neg, r_pos, r_neg = _dual_exp(
                pq[j // 4][0:120, (j % 4) * 128:(j % 4 + 1) * 128], lambda v: after(tk, v))
            eq[j] = (e_pos, e_neg)
            t_pos = jnp.sum(coef[-1, 0] * e_pos, axis=0)
            t_neg = jnp.sum(coef[-1, 1] * e_neg, axis=0)
            rd = 1.0 / (t_pos * r_pos + t_neg * r_neg + 1e-6)
            cq[j] = (r_pos * rd, r_neg * rd)
            due(SLAG, jnp.maximum(cq[j][0], cq[j][1]))

        ngrp = 0
        for d in range(DH):
            for sg in range(2):
                if QS0 <= ngrp < QS0 + NJ:
                    qexp(ngrp - QS0)
                ngrp += 1
                res = es_v[0, :, 256 + sg * 8:264 + sg * 8, :]
                if d == DH - 1:
                    res = _stack([pq[j // 4][120:128, (j % 4) * 128:(j % 4 + 1) * 128]
                                  for j in range(NJ)]) * res
                else:
                    res = es_v[0, :, 272 + d * 8:280 + d * 8, :] * res
                coef[d, sg] = kgroup(sg, res)

        rot.extend((es_v, cj, cr) for cj in range(NJ) for cr in range(0, ER, 8))
        rot.extend((cw_v, cj, cr) for cj in range(15) for cr in range(0, 128, 8))
        for j in range(NJ):
            c_pos, c_neg = cq[j]
            part = []
            for d in range(DH):
                part.append(chain(coef[d, 0], eq[j][0], nrot=2) * c_pos)
                due(PLAG, part[-1])
            for d in range(DH):
                last = part[d] + chain(coef[d, 1], eq[j][1], nrot=2) * c_neg
                ot_v[j, pl.ds(d, 8, stride=16), :] = last
                due(PLAG, last)
            if j % 2 == 1:
                ob = jnp.concatenate([ot_v[j - 1, 0:128, :], ot_v[j, 0:128, :]], axis=1).T
                o_v[g, (j - 1) * 128:(j + 1) * 128, :] = ob.astype(BF)
        assert not rot
        jk = junk[0][1]
        for _, t in junk[1:]:
            jk = jnp.maximum(jk, t)
        junk_v[g] = jk
        return carry

    lax.fori_loop(0, 4, body, 0)

    c_o.wait()
    outs = []
    t0 = 0
    for to in OUT_TILES:
        o = jnp.concatenate([o_v[g, t0:t0 + to, :] for g in range(4)], axis=1)
        a = _dot(o, wo_v[...])
        gt = gt_v[t0:t0 + to, :]
        gt = jnp.concatenate([gt] * 4, axis=1)
        out_v[t0:t0 + to, :] = (gt * a + bb_v[t0:t0 + to, :]).astype(BF)
        co = cp(out_v.at[t0:t0 + to], o_hbm.at[t0:t0 + to], 3)
        co.start()
        outs.append(co)
        t0 += to
    for co in outs:
        co.wait()


@jax.jit
def pallas_gated_mix__linear_kernel_hedgehog__glu_gated_bilinear__prompt_kernel(
    A_x: jax.Array,
    A_wqkv: jax.Array,
    A_w_phi: jax.Array,
    A_wo: jax.Array,
    B_x: jax.Array,
    B_w_gate: jax.Array,
    B_w_up: jax.Array,
    B_w_down: jax.Array,
    gate_w: jax.Array,
):
    del B_x
    x = A_x.reshape(S, D)
    wphi = jnp.transpose(A_w_phi, (1, 2, 0)).reshape(DH * DH, H)
    gw = gate_w.reshape(4, 128)
    any_spec = pl.BlockSpec(memory_space=pl.ANY)
    out = pl.pallas_call(
        _kernel,
        in_specs=[any_spec] * 8,
        out_specs=any_spec,
        out_shape=jax.ShapeDtypeStruct((S, D), BF),
        scratch_shapes=[
            pltpu.VMEM((S, D), BF), pltpu.VMEM((D, 3 * D), BF), pltpu.VMEM((DH * DH, H), BF),
            pltpu.VMEM((D, D), BF), pltpu.VMEM((D, F), BF), pltpu.VMEM((D, F), BF),
            pltpu.VMEM((F, D), BF), pltpu.VMEM((4, 128), BF), pltpu.VMEM((S, D), BF),
            pltpu.VMEM((4, 128, 128), BF),
            pltpu.VMEM((480, D), BF),
            pltpu.VMEM((480, D), BF),
            pltpu.VMEM((4, 8, D), F32),
            pltpu.VMEM((4, D + 16, 128), F32),
            pltpu.VMEM((4, NJ, ER, 128), F32),
            pltpu.VMEM((NJ, 144, 128), F32),
            pltpu.VMEM((4, S, 128), BF),
            pltpu.VMEM((S, D), F32),
            pltpu.VMEM((S, 128), F32),
            pltpu.VMEM((8, 128), F32),
            pltpu.VMEM((4, 8, 128), F32),
            pltpu.VMEM((4, 15, 128, 128), F32),
            pltpu.SemaphoreType.DMA((4,)),
        ],
        compiler_params=pltpu.CompilerParams(vmem_limit_bytes=100 * 1024 * 1024),
    )(x, A_wqkv, wphi, A_wo, B_w_gate, B_w_up, B_w_down, gw)
    return out.reshape(1, S, D)
```
